```python
import jax
import jax.numpy as jnp

def _softmax(x, axis=-1):
    return jax.nn.softmax(x, axis=axis)
def _gelu(x):
    return jax.nn.gelu(x, approximate=True)
def _silu(x):
    return jax.nn.silu(x)
def _sigmoid(x):
    return jax.nn.sigmoid(x)
def _layernorm(x, axis=-1, eps=1e-5):
    m = jnp.mean(x, axis=axis, keepdims=True)
    v = jnp.var(x, axis=axis, keepdims=True)
    return (x - m) / jnp.sqrt(v + eps)
def _scatter_add(tgt, idx, src, axis=0):
    return tgt.at[idx].add(src)
def _segment_sum(src, seg, n):
    return jax.ops.segment_sum(src, seg, n)
class _Rng:
    def __init__(self, key):
        self._k = key
    def _next(self):
        self._k, sub = jax.random.split(self._k)
        return sub
    def normal(self, shape):
        return jax.random.normal(self._next(), shape, dtype=jnp.bfloat16)
    def randint(self, lo, hi, shape):
        return jax.random.randint(self._next(), shape, lo, hi, dtype=jnp.int32)
    def uniform(self, shape, lo=0.0, hi=1.0):
        return jax.random.uniform(self._next(), shape, jnp.bfloat16, lo, hi)
    def permutation(self, n):
        return jax.random.permutation(self._next(), n)


kernel_name = 'interleave_layers__sliding_local_dilated__dense_activation_gelu__prompt'

def setup_inputs():
    _rng = _Rng(jax.random.key(int.from_bytes(__import__("os").urandom(4), "little")))
    _w = (lambda a: (lambda t: t.astype(jnp.bfloat16) if jnp.issubdtype(t.dtype, jnp.floating) else t)(jnp.asarray(a)))
    def _A_setup():
        B, S, D = 1, 2048, 1024
        return {
            "x": _w((lambda *s: _rng.normal(s) * 0.05)(B, S, D)),
            "wqkv": _w((lambda *s: _rng.normal(s) * 0.05)(D, 3 * D)),
            "wo": _w((lambda *s: _rng.normal(s) * 0.05)(D, D)),
        }
    _A_in = _A_setup()

    def _B_setup():
        B, S, D, F = 1, 2048, 1024, 3584
        return {
            "x": _w((lambda *s: _rng.normal(s) * 0.05)(B, S, D)),
            "w1": _w((lambda *s: _rng.normal(s) * 0.05)(D, F) * (D ** -0.5)),
            "b1": _w((lambda *s: _rng.normal(s) * 0.05)(F) * 0.01),
            "w2": _w((lambda *s: _rng.normal(s) * 0.05)(F, D) * (F ** -0.5)),
            "b2": _w((lambda *s: _rng.normal(s) * 0.05)(D) * 0.01),
        }
    _B_in = _B_setup()

    return {
        "A_x": _A_in["x"],
        "A_wqkv": _A_in["wqkv"],
        "A_wo": _A_in["wo"],
        "B_x": _B_in["x"],
        "B_w1": _B_in["w1"],
        "B_b1": _B_in["b1"],
        "B_w2": _B_in["w2"],
        "B_b2": _B_in["b2"],
    }

def reference(A_x, A_wqkv, A_wo, B_x, B_w1, B_b1, B_w2, B_b2):
    def _A_ref(x, wqkv, wo):
        B, S, D = x.shape
        H = 32; Dh = D // H
        W, dil = 8, 2
        qkv = (lambda x, *d: x.transpose(*d))((x @ wqkv).reshape(B, S, 3, H, Dh), 2, 0, 3, 1, 4)
        q, k, v = qkv[0], qkv[1], qkv[2]
        scale = Dh ** -0.5
        pos = jnp.arange(S)
        off = jnp.arange(W) * dil
        idx = pos[:, None] - off[None, :]
        mask = idx >= 0
        idx_c = jnp.where(mask, idx, 0).reshape(-1)
        kg = k[:, :, idx_c, :].reshape(B, H, S, W, Dh)
        vg = v[:, :, idx_c, :].reshape(B, H, S, W, Dh)
        logits = jnp.einsum("bhsd,bhswd->bhsw", q, kg) * scale
        logits = jnp.where(mask[None, None, :, :], logits, -1e9)
        attn = _softmax(logits, axis=-1)
        o = jnp.einsum("bhsw,bhswd->bhsd", attn, vg)
        return (lambda x, *d: x.transpose(*d))(o, 0, 2, 1, 3).reshape(B, S, D) @ wo

    def _B_ref(x, w1, b1, w2, b2):
        h = jnp.einsum("bsd,df->bsf", x, w1) + b1
        h = _gelu(h)
        return jnp.einsum("bsf,fd->bsd", h, w2) + b2

    x = A_x
    x = x + _A_ref(_layernorm(x, axis=-1), A_wqkv, A_wo)
    x = x + _B_ref(_layernorm(x, axis=-1), B_w1, B_b1, B_w2, B_b2)
    x = x + _A_ref(_layernorm(x, axis=-1), A_wqkv, A_wo)
    x = x + _B_ref(_layernorm(x, axis=-1), B_w1, B_b1, B_w2, B_b2)
    return x
```

```python
import functools, math
import jax, jax.numpy as jnp
from jax import lax
import jax.experimental.pallas as pl
import jax.experimental.pallas.tpu as pltpu

S, D, F, H, DH, W, DIL = 2048, 1024, 3584, 32, 32, 8, 2
TM = 256
RC = 8
HALO = 16
NCH = 4
CR = D // NCH
SKEW = 1
GRP = 8
FC = 512
ATTU = 4
MIDWAIT = 2
LC = 16
GATE = 27
QORD = [int(c) for c in "012"]
NT = D // 128
NF = F // 128
NTILE = S // TM
NJOB = 2 * NTILE
EPS = 1e-5
f32, bf16, u32 = jnp.float32, jnp.bfloat16, jnp.uint32

def _ln(x):
    m = jnp.mean(x, axis=-1, keepdims=True)
    xc = x - m
    v = jnp.mean(xc * xc, axis=-1, keepdims=True)
    return xc * lax.rsqrt(v + EPS)

def _gelu(x):
    c = math.sqrt(2.0 / math.pi)
    return 0.5 * x * (1.0 + jnp.tanh(c * (x + 0.044715 * (x * x * x))))

def _dot(a, b):
    return jnp.dot(a, b, preferred_element_type=f32)

def kernel(x_ref, xp_ref, wqkv_hbm, wo_hbm, w1_hbm, b1_ref, w2_hbm, b2_ref, o_ref,
           xs, qkv_s, att_s, xn_s, xn2_s, x2_s, stage, wqkv_ref, wo_ref, w1_ref, w2_ref, sems):
    g = pl.program_id(0)
    c2 = (DH ** -0.5) * math.log2(math.e)

    def slabs(ref, lo, n, rows=slice(None)):
        return jnp.concatenate([ref[lo + j, rows, :] for j in range(n)], axis=1)

    def wslabs(ref, lo, n, rows=slice(None)):
        return pltpu.bitcast(slabs(ref, lo, n, rows), bf16)

    def qk(r0, ws, qs):
        out = []
        for w in ws:
            acc = None
            for j in range(NT):
                t = qs[j] * qkv_s[NT + j, pl.ds(r0 + HALO - DIL * w, RC), :]
                acc = t if acc is None else acc + t
            out.append((acc, pltpu.roll(acc, 64, 1)))
        return out

    def ldq(r0, z=None):
        qs = [qkv_s[j, pl.ds(r0 + HALO, RC), :] for j in range(NT)]
        if z is not None:
            qs = [pltpu.bitcast(pltpu.bitcast(q, u32) | z, f32) for q in qs]
        return qs

    def stB(xs_):
        out = []
        for a, b in xs_:
            s_ = a + b
            out.append((s_, pltpu.roll(s_, 32, 1)))
        return out

    def stCD(r0, xs_, masked):
        ss = []
        for w, (a, b) in enumerate(xs_):
            acc = a + b
            if masked and w > 0:
                pos = (g % NTILE) * TM + r0 + lax.broadcasted_iota(jnp.int32, (RC, 128), 0)
                acc = jnp.where(pos >= DIL * w, acc, -1e9 / (DH ** -0.5))
            ss.append(acc)
        m = functools.reduce(jnp.maximum, ss)
        ps = [jnp.exp2((s - m) * c2) for s in ss]
        den = functools.reduce(lambda a, b: a + b, ps)
        inv = 1.0 / den
        for j in range(NT):
            acc = None
            for w in range(W):
                t = ps[w] * qkv_s[2 * NT + j, pl.ds(r0 + HALO - DIL * w, RC), :]
                acc = t if acc is None else acc + t
            att_s[j, pl.ds(r0, RC), :] = acc * inv

    def attn_rows(base, n, always_mask, grp, skew, gate=None):
        r = lambda c: base + c * RC
        msk = lambda c: always_mask or c * RC < HALO
        if grp:
            for c in range(n):
                qs = ldq(r(c), gate(c) if gate else None)
                res = []
                for w0 in range(0, W, grp):
                    res += stB(qk(r(c), range(w0, min(W, w0 + grp)), qs))
                stCD(r(c), res, msk(c))
            return
        A, B = {}, {}
        for c in range(n + 2 * skew):
            if c < n:
                A[c] = qk(r(c), range(W), ldq(r(c), gate(c) if gate else None))
            if 0 <= c - skew < n:
                B[c - skew] = stB(A.pop(c - skew))
            if 0 <= c - 2 * skew < n:
                cc = c - 2 * skew
                stCD(r(cc), B.pop(cc), msk(cc))

    def cp_qkv(i):
        p, c = i // NCH, i % NCH
        return pltpu.make_async_copy(wqkv_hbm.at[pl.ds(c * CR, CR), pl.ds(p * D, D)], stage.at[i], sems.at[i])
    def cp_wo(c):
        return pltpu.make_async_copy(wo_hbm.at[pl.ds(c * CR, CR), :], stage.at[3 * NCH + c], sems.at[3 * NCH])
    def cp_w1(j):
        return pltpu.make_async_copy(w1_hbm.at[:, pl.ds(j * 128, 128)], w1_ref.bitcast(bf16).at[j], sems.at[3 * NCH + 1])
    def cp_w2(j):
        return pltpu.make_async_copy(w2_hbm.at[:, pl.ds(j * 128, 128)], w2_ref.bitcast(bf16).at[j], sems.at[3 * NCH + 2])
    def wait_w1():
        pltpu.make_async_copy(w1_ref, w1_ref, sems.at[3 * NCH + 1]).wait()
    def wait_w2():
        pltpu.make_async_copy(w2_ref, w2_ref, sems.at[3 * NCH + 2]).wait()

    def barrel(src, u):
        X = [src[(-t) % 8] for t in range(8)]
        for b in (1, 2, 4):
            m = (u & b) != 0
            X = [jnp.where(m, X[(t - b) % 8], X[t]) for t in range(8)]
        return X

    def pmat(t, transposed):
        a = lax.broadcasted_iota(jnp.int32, (128, 128), 1 if transposed else 0)
        b = lax.broadcasted_iota(jnp.int32, (128, 128), 0 if transposed else 1)
        hh, u, j = a >> 5, (a >> 2) & 7, a & 3
        dst = j * 32 + ((u - t) & 7) * 4 + hh
        return jnp.where(dst == b, 1.0, 0.0).astype(bf16)

    def perm_cols(p, c):
        u = (lax.broadcasted_iota(jnp.int32, (CR // 2, 128), 1) >> 2) & 7
        src = [pltpu.bitcast(stage[p * NCH + c, :, s_ * 128:(s_ + 1) * 128], jnp.uint32) for s_ in range(8)]
        Z = barrel(src, u)
        rows = pl.ds(pl.multiple_of(c * (CR // 2), CR // 2), CR // 2)
        for t in range(8):
            y = _dot(pltpu.bitcast(Z[t], bf16), pmat(t, False))
            wqkv_ref[p * NT + t, rows, :] = pltpu.bitcast(y.astype(bf16), u32)

    def perm_rows():
        u = (lax.broadcasted_iota(jnp.int32, (64, 256), 0) >> 1) & 7
        per = CR // 128
        for n in range(D // 256):
            cols = slice(n * 256, (n + 1) * 256)
            src = [pltpu.bitcast(stage[3 * NCH + s_ // per, (s_ % per) * 128:(s_ % per + 1) * 128, cols], jnp.uint32) for s_ in range(8)]
            Z = barrel(src, u)
            for t in range(8):
                y = pltpu.bitcast(_dot(pmat(t, True), pltpu.bitcast(Z[t], bf16)).astype(bf16), u32)
                wo_ref[2 * n, t * 64:(t + 1) * 64, :] = y[:, :128]
                wo_ref[2 * n + 1, t * 64:(t + 1) * 64, :] = y[:, 128:]

    @pl.when(g == 0)
    def _():
        for i in range(NCH):
            cp_qkv(i).start()
        qkv_s[NT:, 0:HALO, :] = jnp.zeros((2 * NT, HALO, 128), f32)
        xv = x_ref[...].astype(f32)
        xn_s[...] = pltpu.bitcast(_ln(xv).astype(bf16), u32)

        def part(p, carry):
            def chunk(c, carry2):
                cp_qkv(p * NCH + c).wait()
                @pl.when(p < 2)
                def _():
                    cp_qkv((p + 1) * NCH + c).start()
                @pl.when(p == 2)
                def _():
                    cp_wo(c).start()
                perm_cols(p, c)
                return carry2
            lax.fori_loop(0, NCH, chunk, 0)
            @pl.when(p == 2)
            def _():
                for j in range(NF):
                    cp_w1(j).start()
            def half(hf, carry2):
                y = _dot(pltpu.bitcast(xn_s[...], bf16), wslabs(wqkv_ref, p * NT + hf * (NT // 2), NT // 2))
                for j in range(NT // 2):
                    qkv_s[p * NT + hf * (NT // 2) + j, HALO:HALO + TM, :] = y[:, j * 128:(j + 1) * 128]
                return carry2
            lax.fori_loop(0, 2, half, 0)
            return carry
        lax.fori_loop(0, 3, part, 0)
        for c in range(NCH):
            cp_wo(c).wait()
        for j in range(NT):
            cp_w2(j).start()
        perm_rows()
        def att(i, carry):
            attn_rows(pl.multiple_of(i * (ATTU * RC), ATTU * RC), ATTU, True, 0, 1)
            return carry
        lax.fori_loop(0, TM // (ATTU * RC), att, 0)
        if not MIDWAIT:
            wait_w1(); wait_w2()

    rp = pl.multiple_of(((g + NTILE - 1) % NTILE) * TM, TM)

    def ln_chunks(load, dst):
        for c in range(TM // LC):
            dst[c * (LC // 2):(c + 1) * (LC // 2), :] = pltpu.bitcast(_ln(load(c * LC)).astype(bf16), u32)

    @pl.when(jnp.logical_and(g > 0, g < NJOB))
    def _():
        xp = jnp.where(g <= NTILE, xp_ref[...].astype(f32), xs[pl.ds(rp, TM), :])
        x2_s[...] = xp + _dot(slabs(att_s, 0, NT).astype(bf16), wslabs(wo_ref, 0, NT))
        r = pl.multiple_of((g % NTILE) * TM, TM)
        ln_chunks(lambda o: jnp.where(g < NTILE, x_ref[o:o + LC, :].astype(f32), xs[pl.ds(r + o, LC), :]), xn_s)
        qkv_s[NT:, 0:HALO, :] = qkv_s[NT:, TM:TM + HALO, :]
        xn1 = pltpu.bitcast(xn_s[...], bf16)
        for p in QORD:
            y = _dot(xn1, wslabs(wqkv_ref, p * NT, NT))
            for j in range(NT):
                qkv_s[p * NT + j, HALO:HALO + TM, :] = y[:, j * 128:(j + 1) * 128]
        ln_chunks(lambda o: x2_s[o:o + LC, :], xn2_s)
        if MIDWAIT:
            @pl.when(g == 1)
            def _():
                wait_w1()
                if MIDWAIT == 2:
                    wait_w2()
        h = _dot(pltpu.bitcast(xn2_s[...], bf16), wslabs(w1_ref, 0, NF)) + b1_ref[...].astype(f32)
        hg = _gelu(h).astype(bf16)
        if MIDWAIT == 1:
            pl.when(g == 1)(wait_w2)
        x3 = x2_s[...] + _dot(hg, wslabs(w2_ref, 0, NT)) + b2_ref[...].astype(f32)
        xs[pl.ds(rp, TM), :] = x3
        o_ref[...] = x3.astype(o_ref.dtype)
        if GATE:
            def gate(c):
                pos = (c * GATE) // 8
                j, i = pos // 4, (pos % 4) * (TM // 4)
                z = pltpu.bitcast(h[i:i + RC, j * 128:(j + 1) * 128], u32)
                return (z >> 31) >> 1
        else:
            gate = None
        attn_rows(0, TM // RC, False, GRP, SKEW, gate)

    @pl.when(g == NJOB)
    def _():
        rows = slice(S - TM, S)
        x2 = xs[rows, :] + _dot(slabs(att_s, 0, NT).astype(bf16), wslabs(wo_ref, 0, NT))
        xn_s[...] = pltpu.bitcast(_ln(x2).astype(bf16), u32)
        xs[rows, :] = x2 + b2_ref[...].astype(f32)
        n = FC // 128
        def ffn(c, carry):
            off = pl.multiple_of(c * FC, FC)
            h = _dot(pltpu.bitcast(xn_s[...], bf16), wslabs(w1_ref, c * n, n)) + b1_ref[:, pl.ds(off, FC)].astype(f32)
            h = _gelu(h).astype(bf16)
            xs[rows, :] += _dot(h, wslabs(w2_ref, 0, NT, pl.ds(pl.multiple_of(c * (FC // 2), FC // 2), FC // 2)))
            return carry
        lax.fori_loop(0, F // FC, ffn, 0)
        o_ref[...] = xs[rows, :].astype(o_ref.dtype)

@jax.jit
def pallas_interleave_layers__sliding_local_dilated__dense_activation_gelu__prompt_kernel(A_x, A_wqkv, A_wo, B_x, B_w1, B_b1, B_w2, B_b2):
    x = A_x.reshape(S, D)
    const = lambda shape: pl.BlockSpec(shape, lambda i: (0, 0))
    anyspec = pl.BlockSpec(memory_space=pl.ANY)
    out = pl.pallas_call(
        kernel,
        grid=(NJOB + 1,),
        in_specs=[pl.BlockSpec((TM, D), lambda g: (jnp.minimum(g, NTILE - 1), 0)), pl.BlockSpec((TM, D), lambda g: (jnp.clip(g - 1, 0, NTILE - 1), 0)), anyspec, anyspec, anyspec, const((1, F)), anyspec, const((1, D))],
        out_specs=pl.BlockSpec((TM, D), lambda g: (jnp.maximum(g - 1 - NTILE, 0), 0)),
        out_shape=jax.ShapeDtypeStruct((S, D), A_x.dtype),
        scratch_shapes=[pltpu.VMEM((S, D), f32), pltpu.VMEM((3 * NT, TM + HALO, 128), f32), pltpu.VMEM((NT, TM, 128), f32), pltpu.VMEM((TM // 2, D), u32), pltpu.VMEM((TM // 2, D), u32), pltpu.VMEM((TM, D), f32),
            pltpu.VMEM((4 * NCH, CR, D), bf16), pltpu.VMEM((3 * NT, D // 2, 128), u32), pltpu.VMEM((NT, D // 2, 128), u32), pltpu.VMEM((NF, D // 2, 128), u32), pltpu.VMEM((NT, F // 2, 128), u32),
            pltpu.SemaphoreType.DMA((3 * NCH + 3,))],
        compiler_params=pltpu.CompilerParams(dimension_semantics=("arbitrary",), vmem_limit_bytes=100 * 1024 * 1024),
    )(x, x, A_wqkv, A_wo, B_w1, B_b1.reshape(1, F), B_w2, B_b2.reshape(1, D))
    return out.reshape(1, S, D)
```

```python
import functools, math
import jax, jax.numpy as jnp
from jax import lax
import jax.experimental.pallas as pl
import jax.experimental.pallas.tpu as pltpu

S, D, F, H, DH, W, DIL = 2048, 1024, 3584, 32, 32, 8, 2
TM = 256
RC = 8
HALO = 16
NCH = 4
CR = D // NCH
SKEW = 1
GRP = 4
FC = 512
LC = 16
FG = [float(int(c, 16)) for c in "01246"]
G1 = 60
G2 = 20
A0 = 28
A1 = 54
NT = D // 128
NF = F // 128
NTILE = S // TM
NJOB = 2 * NTILE
EPS = 1e-5
f32, bf16, u32 = jnp.float32, jnp.bfloat16, jnp.uint32

def _ln(x):
    m = jnp.mean(x, axis=-1, keepdims=True)
    xc = x - m
    v = jnp.mean(xc * xc, axis=-1, keepdims=True)
    return xc * lax.rsqrt(v + EPS)

def _gelu(x):
    c = math.sqrt(2.0 / math.pi)
    return 0.5 * x * (1.0 + jnp.tanh(c * (x + 0.044715 * (x * x * x))))

def _dot(a, b):
    return jnp.dot(a, b, preferred_element_type=f32)

def kernel(x_hbm, wqkv_hbm, wo_hbm, w1_hbm, b1_hbm, w2_hbm, b2_hbm, o_hbm,
           xin, obuf, xs, qkv_s, att_s, xn_s, xn2_s, x2_s, stage, stage_o, pm, b1_v, b2_v, b1_s, b2_s,
           wqkv_ref, wo_ref, w1_ref, w2_ref, sem_x, sem_w, sem_m, sem_o):
    c2 = (DH ** -0.5) * math.log2(math.e)

    def slabs(ref, lo, n, rows=slice(None)):
        return jnp.concatenate([ref[lo + j, rows, :] for j in range(n)], axis=1)

    def wslabs(ref, lo, n, rows=slice(None)):
        return pltpu.bitcast(slabs(ref, lo, n, rows), bf16)

    def qk(r0, ws, qs):
        out = []
        for w in ws:
            acc = None
            for j in range(NT):
                t = qs[j] * qkv_s[NT + j, pl.ds(r0 + HALO - DIL * w, RC), :]
                acc = t if acc is None else acc + t
            out.append((acc, pltpu.roll(acc, 64, 1)))
        return out

    def ldq(r0, z=None):
        qs = [qkv_s[j, pl.ds(r0 + HALO, RC), :] for j in range(NT)]
        if z is not None:
            qs = [pltpu.bitcast(pltpu.bitcast(q, u32) | z, f32) for q in qs]
        return qs

    def stB(xs_):
        out = []
        for a, b in xs_:
            s_ = a + b
            out.append((s_, pltpu.roll(s_, 32, 1)))
        return out

    def stCD(r0, xs_, masked, tile0):
        ss = []
        for w, (a, b) in enumerate(xs_):
            acc = a + b
            if masked and w > 0:
                pos = tile0 + r0 + lax.broadcasted_iota(jnp.int32, (RC, 128), 0)
                acc = jnp.where(pos >= DIL * w, acc, -1e9 / (DH ** -0.5))
            ss.append(acc)
        m = functools.reduce(jnp.maximum, ss)
        ps = [jnp.exp2((s - m) * c2) for s in ss]
        den = functools.reduce(lambda a, b: a + b, ps)
        inv = 1.0 / den
        for j in range(NT):
            acc = None
            for w in range(W):
                t = ps[w] * qkv_s[2 * NT + j, pl.ds(r0 + HALO - DIL * w, RC), :]
                acc = t if acc is None else acc + t
            att_s[j, pl.ds(r0, RC), :] = acc * inv

    def attn_rows(base, n, mode, tile0, grp, skew, gate=None):
        r = lambda c: base + c * RC
        msk = lambda c: mode == 'all' or (mode == 'head' and c * RC < HALO)
        if grp:
            for c in range(n):
                qs = ldq(r(c), gate(c) if gate else None)
                res = []
                for w0 in range(0, W, grp):
                    res += stB(qk(r(c), range(w0, min(W, w0 + grp)), qs))
                stCD(r(c), res, msk(c), tile0)
            return
        A, B = {}, {}
        for c in range(n + 2 * skew):
            if c < n:
                A[c] = qk(r(c), range(W), ldq(r(c), gate(c) if gate else None))
            if 0 <= c - skew < n:
                B[c - skew] = stB(A.pop(c - skew))
            if 0 <= c - 2 * skew < n:
                cc = c - 2 * skew
                stCD(r(cc), B.pop(cc), msk(cc), tile0)

    def cp_x(t):
        rows = pl.ds(pl.multiple_of(t * TM, TM), TM)
        return pltpu.make_async_copy(x_hbm.at[rows, :], xin.at[rows, :], sem_x.at[t])
    def cp_o(t):
        rows = pl.ds(pl.multiple_of(t * TM, TM), TM)
        return pltpu.make_async_copy(obuf.at[rows, :], o_hbm.at[rows, :], sem_o.at[0])
    def cp_qkv(i):
        p, c = i // NCH, i % NCH
        return pltpu.make_async_copy(wqkv_hbm.at[pl.ds(pl.multiple_of(c * CR, CR), CR), pl.ds(pl.multiple_of(p * D, D), D)], stage.at[i], sem_w.at[i])
    def cp_wo(n):
        return pltpu.make_async_copy(wo_hbm.at[:, pl.ds(pl.multiple_of(n * 256, 256), 256)], stage_o.at[n], sem_m.at[0])
    def cp_w1(j):
        return pltpu.make_async_copy(w1_hbm.at[:, pl.ds(j * 128, 128)], w1_ref.bitcast(bf16).at[j], sem_m.at[1])
    W2R = ((0, 2048), (2048, F - 2048))
    def cp_w2(hf, j):
        rows = pl.ds(*W2R[hf])
        return pltpu.make_async_copy(w2_hbm.at[rows, pl.ds(j * 128, 128)], w2_ref.bitcast(bf16).at[j, rows, :], sem_m.at[2 + hf])
    cp_b1 = pltpu.make_async_copy(b1_hbm, b1_v, sem_m.at[4])
    cp_b2 = pltpu.make_async_copy(b2_hbm, b2_v, sem_m.at[5])
    def wait_all(ref, sem):
        pltpu.make_async_copy(ref, ref, sem).wait()
    def wait_w2(hf):
        wait_all(w2_ref.at[:, pl.ds(W2R[hf][0] // 2, W2R[hf][1] // 2), :], sem_m.at[2 + hf])

    def barrel(src, u):
        X = [src[(-t) % 8] for t in range(8)]
        for b in (1, 2, 4):
            m = (u & b) != 0
            X = [jnp.where(m, X[(t - b) % 8], X[t]) for t in range(8)]
        return X

    def pmat(t, transposed):
        a = lax.broadcasted_iota(jnp.int32, (128, 128), 1 if transposed else 0)
        b = lax.broadcasted_iota(jnp.int32, (128, 128), 0 if transposed else 1)
        hh, u, j = a >> 5, (a >> 2) & 7, a & 3
        dst = j * 32 + ((u - t) & 7) * 4 + hh
        return pltpu.bitcast(jnp.where(dst == b, 1.0, 0.0).astype(bf16), u32)

    def perm_cols(p, c):
        u = (lax.broadcasted_iota(jnp.int32, (CR // 2, 128), 1) >> 2) & 7
        src = [pltpu.bitcast(stage[p * NCH + c, :, s_ * 128:(s_ + 1) * 128], u32) for s_ in range(8)]
        Z = barrel(src, u)
        rows = pl.ds(pl.multiple_of(c * (CR // 2), CR // 2), CR // 2)
        for t in range(8):
            l = lax.broadcasted_iota(jnp.int32, (CR // 2, 128), 1)
            idx = (l & 3) * 32 + ((((l >> 2) & 7) + t) & 7) * 4 + (l >> 5)
            wqkv_ref[p * NT + t, rows, :] = jnp.take_along_axis(Z[t], idx, axis=1)

    def perm_rows(n):
        u = (lax.broadcasted_iota(jnp.int32, (64, 256), 0) >> 1) & 7
        src = [pltpu.bitcast(stage_o[n, s_ * 128:(s_ + 1) * 128, :], u32) for s_ in range(8)]
        Z = barrel(src, u)
        for t in range(8):
            y = pltpu.bitcast(_dot(pltpu.bitcast(pm[t], bf16), pltpu.bitcast(Z[t], bf16)).astype(bf16), u32)
            wo_ref[2 * n, t * 64:(t + 1) * 64, :] = y[:, :128]
            wo_ref[2 * n + 1, t * 64:(t + 1) * 64, :] = y[:, 128:]

    def zero_of(v):
        return (pltpu.bitcast(v, u32) >> 31) >> 1

    def ln_chunks(load, dst, lc, gate=None):
        for c in range(TM // lc):
            v = load(c * lc)
            if gate is not None:
                v = pltpu.bitcast(pltpu.bitcast(v, u32) | jnp.tile(gate(c), (lc // RC, NT)), f32)
            dst[c * (lc // 2):(c + 1) * (lc // 2), :] = pltpu.bitcast(_ln(v).astype(bf16), u32)

    def pick(tiles, t):
        j = int(t)
        i = int((t - j) * (TM // RC)) * RC
        return zero_of(tiles[j][i:i + RC, :])

    def cols(y):
        return [y[:, j * 128:(j + 1) * 128] for j in range(y.shape[1] // 128)]

    cp_qkv(0).start(); cp_x(0).start(); cp_qkv(1).start()
    def mk(t, c):
        pm[t] = pmat(t, True)
        return c
    lax.fori_loop(0, 8, mk, 0)
    qkv_s[NT:, TM:TM + HALO, :] = jnp.zeros((2 * NT, HALO, 128), f32)

    def starts(cp, lo, hi):
        def st(j, c):
            cp(j).start()
            return c
        lax.fori_loop(lo, hi, st, 0)
    def g0():
        starts(cp_qkv, 7, 10)
    def g1():
        starts(cp_qkv, 10, 12)
    def g2():
        starts(cp_wo, 0, 3)
    def g3():
        cp_wo(3).start(); cp_x(1).start(); cp_b1.start(); cp_b2.start()
        starts(cp_w1, 0, 2)
    def g4():
        starts(cp_w1, 2, 8)
    def g5():
        starts(cp_w1, 8, 16)
    groups = [g0, g1, g2, g3, g4, g5]

    def step(g, carry):
        tp = (g + NTILE - 1) % NTILE
        rp = pl.multiple_of(tp * TM, TM)
        r = pl.multiple_of((g % NTILE) * TM, TM)
        edge = jnp.logical_or(g == 1, g == NJOB)

        @pl.when(g < NTILE)
        def _():
            cp_x(g).wait()

        @pl.when(g == 0)
        def _():
            cp_qkv(2).start()

        def x_prev():
            return jnp.where(g <= NTILE, xin[pl.ds(rp, TM), :].astype(f32), xs[pl.ds(rp, TM), :])

        @pl.when(edge)
        def _():
            x2 = x_prev() + _dot(slabs(att_s, 0, NT).astype(bf16), wslabs(wo_ref, 0, NT))
            xn2_s[...] = pltpu.bitcast(_ln(x2).astype(bf16), u32)
            xs[pl.ds(rp, TM), :] = x2 + b2_s[...]

        @pl.when(g <= 1)
        def _():
            xn_s[...] = pltpu.bitcast(_ln(xin[pl.ds(r, TM), :].astype(f32)).astype(bf16), u32)
            qkv_s[NT:, 0:HALO, :] = qkv_s[NT:, TM:TM + HALO, :]
            @pl.when(g == 0)
            def _():
                def chunk(c, c2_):
                    cp_qkv(c).wait()
                    cp_qkv(c + 3).start()
                    perm_cols(0, c)
                    return c2_
                lax.fori_loop(0, NCH, chunk, 0)
            def half(i, c2_):
                @pl.when(jnp.logical_and(g == 0, i < 4))
                def _():
                    cp_qkv(NCH + 2 * i).wait()
                    cp_qkv(NCH + 2 * i + 1).wait()
                for k, grp in enumerate(groups):
                    pl.when(jnp.logical_and(g == 0, i == k))(grp)
                y = _dot(pltpu.bitcast(xn_s[...], bf16), wslabs(wqkv_ref, i * 4, 4))
                for j in range(4):
                    qkv_s[i * 4 + j, HALO:HALO + TM, :] = y[:, j * 128:(j + 1) * 128]
                pn = (i // 2 + 1) % 3
                perm_cols(pn, 2 * (i % 2))
                perm_cols(pn, 2 * (i % 2) + 1)
                return c2_
            lax.fori_loop(0, 6, half, 0)

        @pl.when(g == 0)
        def _():
            starts(cp_w1, 16, NF)
            wait_all(stage_o, sem_m.at[0])
            cp_b1.wait(); cp_b2.wait()
            b1_s[...] = b1_v[...].astype(f32).reshape(1, F)
            b2_s[...] = b2_v[...].astype(f32).reshape(1, D)
            def att(n, c1):
                perm_rows(n)
                attn_rows(pl.multiple_of(n * (TM // 4), TM // 4), TM // 4 // RC, 'all', 0, 0, 1)
                return c1
            lax.fori_loop(0, 4, att, 0)
            starts(lambda j: cp_w2(0, j), 0, NT)
            starts(lambda j: cp_w2(1, j), 0, NT)

        @pl.when(g == 1)
        def _():
            starts(cp_x, 2, NTILE)

        @pl.when(edge)
        def _():
            n = FC // 128
            nit = F // FC
            na = -(-(TM // RC) // nit)
            def ffn(c, c1):
                @pl.when(jnp.logical_and(g == 1, c == 0))
                def _():
                    wait_all(w1_ref, sem_m.at[1])
                    wait_w2(0)
                @pl.when(jnp.logical_and(g == 1, c == W2R[1][0] // FC))
                def _():
                    wait_w2(1)
                off = pl.multiple_of(c * FC, FC)
                h = _dot(pltpu.bitcast(xn2_s[...], bf16), wslabs(w1_ref, c * n, n)) + b1_s[:, pl.ds(off, FC)]
                hg = _gelu(h).astype(bf16)
                y = _dot(hg, wslabs(w2_ref, 0, NT, pl.ds(pl.multiple_of(c * (FC // 2), FC // 2), FC // 2)))
                x3 = xs[pl.ds(rp, TM), :] + y
                xs[pl.ds(rp, TM), :] = x3
                obuf[pl.ds(rp, TM), :] = x3.astype(bf16)
                tl = cols(h) + cols(y)
                base = pl.multiple_of(jnp.minimum(c * na, TM // RC - na) * RC, RC)
                attn_rows(base, na, 'none', 0, GRP, SKEW, lambda k: pick(tl, FG[k]))
                return c1
            lax.fori_loop(0, nit, ffn, 0)

        @pl.when(jnp.logical_and(g > 1, g < NJOB))
        def _():
            yo = _dot(slabs(att_s, 0, NT).astype(bf16), wslabs(wo_ref, 0, NT))
            x2_s[...] = x_prev() + yo
            yos = cols(yo)
            nl = TM // LC
            ln_chunks(lambda o: jnp.where(g < NTILE, xin[pl.ds(r + o, LC), :].astype(f32), xs[pl.ds(r + o, LC), :]), xn_s, LC,
                      lambda c: pick(yos, c * G1 / 10 / nl))
            qkv_s[NT:, 0:HALO, :] = qkv_s[NT:, TM:TM + HALO, :]
            ys = cols(_dot(pltpu.bitcast(xn_s[...], bf16), wslabs(wqkv_ref, 0, 3 * NT)))
            for j in range(3 * NT):
                qkv_s[j, HALO:HALO + TM, :] = ys[j]
            ln_chunks(lambda o: x2_s[o:o + LC, :], xn2_s, LC, lambda c: pick(ys, c * G2 / nl))
            h = _dot(pltpu.bitcast(xn2_s[...], bf16), wslabs(w1_ref, 0, NF)) + b1_s[...]
            hg = _gelu(h).astype(bf16)
            tl = cols(h)
            outs = []
            for j in range(NT):
                acc = None
                for k in range(F // 512):
                    t = _dot(hg[:, k * 512:(k + 1) * 512], wslabs(w2_ref, j, 1, slice(k * 256, (k + 1) * 256)))
                    acc = t if acc is None else acc + t
                    if (j * 7 + k) % 2 == 1:
                        tl.append(acc)
                outs.append(acc)
            x3 = x2_s[...] + jnp.concatenate(outs, axis=1) + b2_s[...]
            xs[pl.ds(rp, TM), :] = x3
            obuf[pl.ds(rp, TM), :] = x3.astype(bf16)
            na = TM // RC
            attn_rows(0, na, 'head', r, GRP, SKEW, lambda c: pick(tl, A0 + c * (A1 - A0) / na))

        @pl.when(g > NTILE)
        def _():
            cp_o(tp).start()
        return carry

    lax.fori_loop(0, NJOB + 1, step, 0)
    wait_all(obuf, sem_o.at[0])

@jax.jit
def pallas_interleave_layers__sliding_local_dilated__dense_activation_gelu__prompt_kernel(A_x, A_wqkv, A_wo, B_x, B_w1, B_b1, B_w2, B_b2):
    x = A_x.reshape(S, D)
    anyspec = pl.BlockSpec(memory_space=pl.ANY)
    V = pltpu.VMEM
    out = pl.pallas_call(
        kernel,
        in_specs=[anyspec] * 7,
        out_specs=anyspec,
        out_shape=jax.ShapeDtypeStruct((S, D), A_x.dtype),
        scratch_shapes=[V((S, D), bf16), V((S, D), bf16), V((S, D), f32), V((3 * NT, TM + HALO, 128), f32), V((NT, TM, 128), f32),
            V((TM // 2, D), u32), V((TM // 2, D), u32), V((TM, D), f32),
            V((3 * NCH, CR, D), bf16), V((4, D, 256), bf16), V((8, 64, 128), u32), V((F,), bf16), V((D,), bf16), V((1, F), f32), V((1, D), f32),
            V((3 * NT, D // 2, 128), u32), V((NT, D // 2, 128), u32), V((NF, D // 2, 128), u32), V((NT, F // 2, 128), u32),
            pltpu.SemaphoreType.DMA((NTILE,)), pltpu.SemaphoreType.DMA((3 * NCH,)), pltpu.SemaphoreType.DMA((6,)), pltpu.SemaphoreType.DMA((1,))],
        compiler_params=pltpu.CompilerParams(vmem_limit_bytes=100 * 1024 * 1024),
    )(x, A_wqkv, A_wo, B_w1, B_b1, B_w2, B_b2)
    return out.reshape(1, S, D)
```

```python
import functools, math
import jax, jax.numpy as jnp
from jax import lax
import jax.experimental.pallas as pl
import jax.experimental.pallas.tpu as pltpu

S, D, F, H, DH, W, DIL = 2048, 1024, 3584, 32, 32, 8, 2
TM = 256
RC = 8
HALO = 16
NCH = 4
CR = D // NCH
SKEW = 1
GRP = 4
FC = 896
LC = 16
AG = 70
AO = 60
F0 = 1
FD = 150
SUB = (25, 50, 75, 2, 1)
G1 = 60
G2 = 20
A0 = 2
A1 = 54
NT = D // 128
NF = F // 128
NTILE = S // TM
NJOB = 2 * NTILE
EPS = 1e-5
f32, bf16, u32 = jnp.float32, jnp.bfloat16, jnp.uint32

def _ln(x):
    m = jnp.mean(x, axis=-1, keepdims=True)
    xc = x - m
    v = jnp.mean(xc * xc, axis=-1, keepdims=True)
    return xc * lax.rsqrt(v + EPS)

def _gelu(x):
    c = math.sqrt(2.0 / math.pi)
    return 0.5 * x * (1.0 + jnp.tanh(c * (x + 0.044715 * (x * x * x))))

def _dot(a, b):
    return jnp.dot(a, b, preferred_element_type=f32)

def kernel(x_hbm, wqkv_hbm, wo_hbm, w1_hbm, b1_hbm, w2_hbm, b2_hbm, o_hbm,
           xin, obuf, xs, qkv_s, qkv0_s, att_s, xn_s, xn2_s, x2_s, stage, stage_o, b1_v, b2_v, b1_s, b2_s,
           wqkv_ref, wo_ref, w1_ref, w2_ref, sem_x, sem_w, sem_m, sem_f, sem_o):
    c2 = (DH ** -0.5) * math.log2(math.e)

    def slabs(ref, lo, n, rows=slice(None)):
        return jnp.concatenate([ref[lo + j, rows, :] for j in range(n)], axis=1)

    def wslabs(ref, lo, n, rows=slice(None)):
        return pltpu.bitcast(slabs(ref, lo, n, rows), bf16)

    def qk(Q, r0, ws, qs):
        out = []
        for w in ws:
            acc = None
            for j in range(NT):
                t = qs[j] * Q[NT + j, pl.ds(r0 + HALO - DIL * w, RC), :]
                acc = t if acc is None else acc + t
            out.append((acc, pltpu.roll(acc, 64, 1)))
        return out

    def ldq(Q, r0, z=None):
        qs = [Q[j, pl.ds(r0 + HALO, RC), :] for j in range(NT)]
        if z is not None:
            qs = [pltpu.bitcast(pltpu.bitcast(q, u32) | z, f32) for q in qs]
        return qs

    def stB(xs_):
        out = []
        for a, b in xs_:
            s_ = a + b
            out.append((s_, pltpu.roll(s_, 32, 1)))
        return out

    def stCD(Q, r0, xs_, masked, tile0, pg=None):
        ss = []
        for w, (a, b) in enumerate(xs_):
            acc = a + b
            if masked and w > 0:
                pos = tile0 + r0 + lax.broadcasted_iota(jnp.int32, (RC, 128), 0)
                acc = jnp.where(pos >= DIL * w, acc, -1e9 / (DH ** -0.5))
            ss.append(acc)
        m = functools.reduce(jnp.maximum, ss)
        ps = [jnp.exp2((s - m) * c2) for s in ss]
        den = functools.reduce(lambda a, b: a + b, ps)
        inv = 1.0 / den
        for j in range(NT):
            acc = None
            if pg is not None and pg(j) is not None:
                ps = [pltpu.bitcast(pltpu.bitcast(p_, u32) | pg(j), f32) for p_ in ps]
            for w in range(W):
                t = ps[w] * Q[2 * NT + j, pl.ds(r0 + HALO - DIL * w, RC), :]
                acc = t if acc is None else acc + t
            att_s[j, pl.ds(r0, RC), :] = acc * inv

    def attn_rows(Q, base, n, mode, tile0, grp, skew, gate=None, sub=None):
        r = lambda c: base + c * RC
        msk = lambda c: mode == 'all' or (mode == 'head' and c * RC < HALO)
        if grp:
            for c in range(n):
                qs = ldq(Q, r(c), gate(c) if gate else None)
                res = []
                for w0 in range(0, W, grp):
                    if sub and w0 and sub[0]:
                        qs = ldq(Q, r(c), gate(c + sub[0] * w0 / 4 / 100))
                    res += stB(qk(Q, r(c), range(w0, min(W, w0 + grp)), qs))
                pg = None
                if sub:
                    pg = lambda j: gate(c + (sub[1] + (sub[2] - sub[1]) * j / 4) / 100) if j % sub[3] == 0 and j >= sub[4] else None
                stCD(Q, r(c), res, msk(c), tile0, pg)
            return
        A, B = {}, {}
        for c in range(n + 2 * skew):
            if c < n:
                A[c] = qk(Q, r(c), range(W), ldq(Q, r(c), gate(c) if gate else None))
            if 0 <= c - skew < n:
                B[c - skew] = stB(A.pop(c - skew))
            if 0 <= c - 2 * skew < n:
                cc = c - 2 * skew
                stCD(Q, r(cc), B.pop(cc), msk(cc), tile0)

    def cp_x(t):
        rows = pl.ds(pl.multiple_of(t * TM, TM), TM)
        return pltpu.make_async_copy(x_hbm.at[rows, :], xin.at[rows, :], sem_x.at[0])
    def cp_o(t):
        rows = pl.ds(pl.multiple_of(t * TM, TM), TM)
        return pltpu.make_async_copy(obuf.at[rows, :], o_hbm.at[rows, :], sem_o.at[0])
    def cp_qkv(i, sem=None):
        p, c = i // NCH, i % NCH
        return pltpu.make_async_copy(wqkv_hbm.at[pl.ds(pl.multiple_of(c * CR, CR), CR), pl.ds(pl.multiple_of(p * D, D), D)], stage.at[i],
                                     sem_w.at[(i // 2) % 3 if sem is None else sem])
    def cp_wo(n):
        return pltpu.make_async_copy(wo_hbm.at[:, pl.ds(pl.multiple_of(n * 128, 128), 128)], stage_o.bitcast(bf16).at[n, 0:D, :], sem_m.at[n // 2])
    FGR = ((0, 2), (2, 4), (4, 7)) if FC == 512 else ((0, 1), (1, 2), (2, 4))
    def cp_w1(gr, j):
        return pltpu.make_async_copy(w1_hbm.at[:, pl.ds(j * 128, 128)], w1_ref.bitcast(bf16).at[j], sem_f.at[gr])
    def cp_w2(gr, j):
        rows = pl.ds(FGR[gr][0] * FC, (FGR[gr][1] - FGR[gr][0]) * FC)
        return pltpu.make_async_copy(w2_hbm.at[rows, pl.ds(j * 128, 128)], w2_ref.bitcast(bf16).at[j, rows, :], sem_f.at[gr])
    cp_b1 = pltpu.make_async_copy(b1_hbm, b1_v, sem_m.at[4])
    cp_b2 = pltpu.make_async_copy(b2_hbm, b2_v, sem_m.at[4])
    def wait_all(ref, sem):
        pltpu.make_async_copy(ref, ref, sem).wait()
    def wait_f(gr):
        lo, n = FGR[gr][0], FGR[gr][1] - FGR[gr][0]
        wait_all(w1_ref.at[pl.ds(lo * FC // 128, n * FC // 128)], sem_f.at[gr])
        wait_all(w2_ref.at[:, pl.ds(lo * FC // 2, n * FC // 2), :], sem_f.at[gr])

    def barrel(src, u):
        X = [src[(-t) % 8] for t in range(8)]
        for b in (1, 2, 4):
            m = (u & b) != 0
            X = [jnp.where(m, X[(t - b) % 8], X[t]) for t in range(8)]
        return X

    PR = 8
    def perm_cols(i, PR, gate=None):
        p, c = i // NCH, i % NCH
        l = lax.broadcasted_iota(jnp.int32, (PR, 128), 1)
        u = (l >> 2) & 7
        for rb in range(CR // 2 // PR):
            src = [pltpu.bitcast(stage[i, 2 * PR * rb:2 * PR * (rb + 1), s_ * 128:(s_ + 1) * 128], u32) for s_ in range(8)]
            z = gate(rb) if gate else None
            if z is not None:
                src = [v | jnp.tile(z, (PR // RC, 1)) for v in src]
            Z = barrel(src, u)
            rows = pl.ds(pl.multiple_of(c * (CR // 2) + rb * PR, PR), PR)
            for t in range(8):
                idx = (l & 3) * 32 + ((u + t) & 7) * 4 + (l >> 5)
                wqkv_ref[p * NT + t, rows, :] = jnp.take_along_axis(Z[t], idx, axis=1)

    def perm_rows(n, gate):
        sub = lax.broadcasted_iota(jnp.int32, (8, 128), 0)
        def ld(base, o):
            v = stage_o[n, base + o:base + o + 8, :]
            if o > 8:
                v = jnp.where(sub < 16 - o, v, stage_o[n, base + o - 16:base + o - 8, :])
            return v
        for s_ in range(8):
            for hp in range(2):
                for m in range(2):
                    o = (2 * s_ + 8 * m) % 16
                    a_, b_ = ld(s_ * 64 + hp * 32, o), ld(s_ * 64 + hp * 32 + 16, o)
                    z = gate(s_ * 4 + hp * 2 + m)
                    if z is not None:
                        a_ = a_ | z
                    d0 = m * 256 + s_ * 2 + hp
                    wo_ref[n, pl.ds(d0, 8, stride=32), :] = (a_ & 0xffff) | (b_ << 16)
                    wo_ref[n, pl.ds(d0 + 16, 8, stride=32), :] = (a_ >> 16) | ((b_ >> 16) << 16)

    def zero_of(v):
        return (pltpu.bitcast(v, u32) >> 31) >> 1

    def ln_chunks(load, dst, lc, gate=None):
        for c in range(TM // lc):
            v = load(c * lc)
            if gate is not None:
                v = pltpu.bitcast(pltpu.bitcast(v, u32) | jnp.tile(gate(c), (lc // RC, NT)), f32)
            dst[c * (lc // 2):(c + 1) * (lc // 2), :] = pltpu.bitcast(_ln(v).astype(bf16), u32)

    def pick(tiles, t):
        j = int(t)
        i = int((t - j) * (TM // RC)) * RC
        return zero_of(tiles[j][i:i + RC, :])

    def cols(y):
        return [y[:, j * 128:(j + 1) * 128] for j in range(y.shape[1] // 128)]

    def starts(cp, lo, hi):
        for j in range(lo, hi):
            cp(j).start()
    def start_f1(gr):
        starts(lambda j: cp_w1(gr, j), FGR[gr][0] * FC // 128, FGR[gr][1] * FC // 128)
    def start_f2(gr):
        starts(lambda j: cp_w2(gr, j), 0, NT)

    cp_qkv(0).start(); cp_x(0).start(); cp_qkv(1, 3).start()
    qkv0_s[NT:, 0:HALO, :] = jnp.zeros((2 * NT, HALO, 128), f32)
    cp_x(0).wait()
    starts(cp_qkv, 2, 4)
    xn_s[...] = pltpu.bitcast(_ln(xin[0:TM, :].astype(f32)).astype(bf16), u32)
    NK = 2
    CI = NCH // NK
    NI = 3 * NK
    LA = 6
    def chunk(c, c2_):
        cp_qkv(c, 3 * c).wait()
        if LA > 4:
            cp_qkv(c + 4).start()
        perm_cols(c, CR // 2)
        return c2_
    if CI == 1:
        chunk(0, 0)
    else:
        lax.fori_loop(0, CI, chunk, 0)

    LI = 4
    LR = TM // (NI - LI)
    XI = 2
    WI = 3
    def grp(k):
        starts(cp_qkv, CI * k + LA, min(CI * k + LA + CI, 3 * NCH))
        if k == XI:
            cp_x(1).start()
        if WI <= k < WI + NK:
            starts(cp_wo, (k - WI) * 2 * CI, (k - WI + 1) * 2 * CI)
        if k == WI:
            cp_b1.start(); cp_b2.start()
        if k == NI - 2:
            start_f1(0)
        if k == NI - 1:
            start_f2(0)
    def wgrp(k):
        wait_all(stage.at[2 * k + 2:2 * k + 4], sem_w.at[(k + 1) % 3])
        if k == LI:
            cp_x(1).wait()
    def starts_half(i):
        for k in range(NI):
            pl.when(i == k)(functools.partial(grp, k))
    def half(i, c2_):
        for k in range(NI - 1):
            pl.when(i == k)(functools.partial(wgrp, k))
        if 1 == 0:
            starts_half(i)
        p, kh = i // NK, i % NK
        y = _dot(pltpu.bitcast(xn_s[:, pl.ds(pl.multiple_of(kh * (D // NK), D // NK), D // NK)], bf16),
                 wslabs(wqkv_ref, p * NT, NT, pl.ds(pl.multiple_of(kh * (D // NK // 2), D // NK // 2), D // NK // 2)))
        for j in range(NT):
            old = jnp.where(kh == 0, 0.0, qkv0_s[p * NT + j, HALO:HALO + TM, :])
            qkv0_s[p * NT + j, HALO:HALO + TM, :] = old + y[:, j * 128:(j + 1) * 128]
        if 1 == 1:
            starts_half(i)
        ys = cols(y)
        def gt(f, span, off):
            t = f * span / 10 - off / 10
            return pick(ys, t) if t >= 0 else None
        nb = CR // 2 // PR
        for c in range(CI):
            perm_cols((CI * (i + 1) + c) % (3 * NCH), PR, lambda rb: gt((c * nb + rb) / (CI * nb), 75, 10))
        src = pl.multiple_of(jnp.where(i < LI, 0, TM + (i - LI) * LR), LR)
        dst = pl.multiple_of(jnp.maximum(i - LI, 0) * (LR // 2), LR // 2)
        for c in range(LR // LC):
            v = xin[pl.ds(src + c * LC, LC), :].astype(f32)
            z = gt(c / (LR // LC), 70, 10)
            if z is not None:
                v = pltpu.bitcast(pltpu.bitcast(v, u32) | jnp.tile(z, (LC // RC, NT)), f32)
            xn2_s[pl.ds(dst + c * (LC // 2), LC // 2), :] = pltpu.bitcast(_ln(v).astype(bf16), u32)
        return c2_
    lax.fori_loop(0, NI, half, 0)

    cp_b1.wait(); cp_b2.wait()
    b1_s[...] = b1_v[...].astype(f32).reshape(1, F)
    b2_s[...] = b2_v[...].astype(f32).reshape(1, D)
    qkv_s[NT:, 0:HALO, :] = qkv0_s[NT:, TM:TM + HALO, :]
    def grp2(k):
        if k == 0:
            start_f1(1); start_f2(1)
        if k == 1:
            start_f1(2)
        if k == 2:
            start_f2(2)
        if k == 3:
            starts(cp_x, 2, NTILE)
    def att(n, c1):
        wait_all(stage_o.at[pl.ds(2 * n, 2), 0:D // 2, :], sem_m.at[n])
        y = cols(_dot(pltpu.bitcast(xn2_s[...], bf16), wslabs(wqkv_ref, n * 6, 6)))
        for j in range(6):
            qkv_s[n * 6 + j, HALO:HALO + TM, :] = y[j]
        for k in range(4):
            pl.when(n == k)(functools.partial(grp2, k))
        PG = 55 / 10
        tq = lambda q: q // 2 * 2 * PG / 64 - 6 / 10
        for e in range(2):
            perm_rows(2 * n + e, lambda q: pick(y, tq(q + 32 * e)) if tq(q + 32 * e) >= 0 else None)
        attn_rows(qkv0_s, pl.multiple_of(n * (TM // 4), TM // 4), TM // 4 // RC, 'head', 0, GRP, SKEW,
                  lambda k: pick(y, (k * AG - AO) / 100) if k * AG >= AO else None, SUB if 1 else None)
        return c1
    lax.fori_loop(0, 4, att, 0)

    def step(g, carry):
        tp = (g + NTILE - 1) % NTILE
        rp = pl.multiple_of(tp * TM, TM)
        r = pl.multiple_of((g % NTILE) * TM, TM)
        edge = jnp.logical_or(g == 1, g == NJOB)

        def out_prev():
            @pl.when(g > NTILE + 1)
            def _():
                cp_o(g - NTILE - 2).start()

        def x_prev():
            return jnp.where(g <= NTILE, xin[pl.ds(rp, TM), :].astype(f32), xs[pl.ds(rp, TM), :])

        @pl.when(edge)
        def _():
            out_prev()
            for lo in (0, TM // 2):
                rows = pl.ds(rp + lo, TM // 2)
                xp = jnp.where(g <= NTILE, xin[rows, :].astype(f32), xs[rows, :])
                x2 = xp + _dot(slabs(att_s, 0, NT, slice(lo, lo + TM // 2)).astype(bf16), wslabs(wo_ref, 0, NT))
                xn2_s[lo // 2:lo // 2 + TM // 4, :] = pltpu.bitcast(_ln(x2).astype(bf16), u32)
                xs[rows, :] = x2 + b2_s[...]

        @pl.when(edge)
        def _():
            n = FC // 128
            nit = F // FC
            na = -(-(TM // RC) // nit)
            def ffn(c, c1):
                for gr in range(3):
                    pl.when(jnp.logical_and(g == 1, c == FGR[gr][0]))(functools.partial(wait_f, gr))
                @pl.when(jnp.logical_and(g == 1, c == nit - 1))
                def _():
                    wait_all(xin.at[2 * TM:S, :], sem_x.at[0])
                off = pl.multiple_of(c * FC, FC)
                h = _dot(pltpu.bitcast(xn2_s[...], bf16), wslabs(w1_ref, c * n, n)) + b1_s[:, pl.ds(off, FC)]
                hg = _gelu(h).astype(bf16)
                y = _dot(hg, wslabs(w2_ref, 0, NT, pl.ds(pl.multiple_of(c * (FC // 2), FC // 2), FC // 2)))
                x3 = xs[pl.ds(rp, TM), :] + y
                xs[pl.ds(rp, TM), :] = x3
                obuf[pl.ds(rp, TM), :] = x3.astype(bf16)
                tl = cols(h) + cols(y)
                base = pl.multiple_of(jnp.minimum(c * na, TM // RC - na) * RC, RC)
                attn_rows(qkv_s, base, na, 'none', 0, GRP, SKEW, lambda k: pick(tl, F0 + k * FD / 100), SUB if 1 else None)
                return c1
            lax.fori_loop(0, nit, ffn, 0)

        @pl.when(jnp.logical_and(g > 1, g < NJOB))
        def _():
            if 1 == 0:
                out_prev()
            yo = _dot(slabs(att_s, 0, NT).astype(bf16), wslabs(wo_ref, 0, NT))
            x2_s[...] = x_prev() + yo
            yos = cols(yo)
            nl = TM // LC
            ln_chunks(lambda o: jnp.where(g < NTILE, xin[pl.ds(r + o, LC), :].astype(f32), xs[pl.ds(r + o, LC), :]), xn_s, LC,
                      lambda c: pick(yos, c * G1 / 10 / nl))
            qkv_s[NT:, 0:HALO, :] = qkv_s[NT:, TM:TM + HALO, :]
            ys = cols(_dot(pltpu.bitcast(xn_s[...], bf16), wslabs(wqkv_ref, 0, 3 * NT)))
            for j in range(3 * NT):
                qkv_s[j, HALO:HALO + TM, :] = ys[j]
            ln_chunks(lambda o: x2_s[o:o + LC, :], xn2_s, LC, lambda c: pick(ys, c * G2 / nl))
            if 1 == 1:
                out_prev()
            h = _dot(pltpu.bitcast(xn2_s[...], bf16), wslabs(w1_ref, 0, NF)) + b1_s[...]
            hg = _gelu(h).astype(bf16)
            tl = cols(h)
            outs = []
            for j in range(NT):
                acc = None
                for k in range(F // 512):
                    t = _dot(hg[:, k * 512:(k + 1) * 512], wslabs(w2_ref, j, 1, slice(k * 256, (k + 1) * 256)))
                    acc = t if acc is None else acc + t
                    if (j * 7 + k) % 2 == 1:
                        tl.append(acc)
                outs.append(acc)
            x3 = x2_s[...] + jnp.concatenate(outs, axis=1) + b2_s[...]
            xs[pl.ds(rp, TM), :] = x3
            obuf[pl.ds(rp, TM), :] = x3.astype(bf16)
            na = TM // RC
            attn_rows(qkv_s, 0, na, 'head', r, GRP, SKEW, lambda c: pick(tl, A0 + c * (A1 - A0) / na), SUB)

        return carry

    lax.fori_loop(1, NJOB + 1, step, 0)
    cp_o(NTILE - 1).start()
    wait_all(obuf, sem_o.at[0])

@jax.jit
def pallas_interleave_layers__sliding_local_dilated__dense_activation_gelu__prompt_kernel(A_x, A_wqkv, A_wo, B_x, B_w1, B_b1, B_w2, B_b2):
    x = A_x.reshape(S, D)
    anyspec = pl.BlockSpec(memory_space=pl.ANY)
    V = pltpu.VMEM
    out = pl.pallas_call(
        kernel,
        in_specs=[anyspec] * 7,
        out_specs=anyspec,
        out_shape=jax.ShapeDtypeStruct((S, D), A_x.dtype),
        scratch_shapes=[V((S, D), bf16), V((S, D), bf16), V((S, D), f32), V((3 * NT, TM + HALO, 128), f32), V((3 * NT, TM + HALO, 128), f32), V((NT, TM, 128), f32),
            V((TM // 2, D), u32), V((TM // 2, D), u32), V((TM, D), f32),
            V((3 * NCH, CR, D), bf16), V((NT, D // 2 + 8, 128), u32), V((F,), bf16), V((D,), bf16), V((1, F), f32), V((1, D), f32),
            V((3 * NT, D // 2, 128), u32), V((NT, D // 2, 128), u32), V((NF, D // 2, 128), u32), V((NT, F // 2, 128), u32),
            pltpu.SemaphoreType.DMA((1,)), pltpu.SemaphoreType.DMA((4,)), pltpu.SemaphoreType.DMA((5,)), pltpu.SemaphoreType.DMA((3,)), pltpu.SemaphoreType.DMA((1,))],
        compiler_params=pltpu.CompilerParams(vmem_limit_bytes=100 * 1024 * 1024),
    )(x, A_wqkv, A_wo, B_w1, B_b1, B_w2, B_b2)
    return out.reshape(1, S, D)
```

```python
import functools, math
import jax, jax.numpy as jnp
from jax import lax
import jax.experimental.pallas as pl
import jax.experimental.pallas.tpu as pltpu

S, D, F, H, DH, W, DIL = 2048, 1024, 3584, 32, 32, 8, 2
TM = 256
RC = 8
HALO = 16
NCH = 4
CR = D // NCH
SKEW = 1
GRP = 4
FC = 896
LC = 16
OC = [128 * int(c) for c in "0578"]
AG = 70
AO = 60
F0 = 1
FD = 150
SUB = (25, 50, 75, 2, 1)
G1 = 60
G2 = 20
A0 = 2
A1 = 54
NT = D // 128
NF = F // 128
NTILE = S // TM
NJOB = 2 * NTILE
EPS = 1e-5
f32, bf16, u32 = jnp.float32, jnp.bfloat16, jnp.uint32

def _ln(x):
    m = jnp.mean(x, axis=-1, keepdims=True)
    xc = x - m
    v = jnp.mean(xc * xc, axis=-1, keepdims=True)
    return xc * lax.rsqrt(v + EPS)

def _gelu(x):
    c = math.sqrt(2.0 / math.pi)
    return 0.5 * x * (1.0 + jnp.tanh(c * (x + 0.044715 * (x * x * x))))

def _dot(a, b):
    return jnp.dot(a, b, preferred_element_type=f32)

def kernel(x_hbm, wqkv_hbm, wo_hbm, w1_hbm, b1_hbm, w2_hbm, b2_hbm, o_hbm,
           xin, obuf, xs, qkv_s, qkv0_s, att_s, xn_s, xn2_s, x2_s, stage, stage_o, b1_v, b2_v, b1_s, b2_s,
           wqkv_ref, wo_ref, w1_ref, w2_ref, sem_x, sem_w, sem_m, sem_f, sem_o):
    c2 = (DH ** -0.5) * math.log2(math.e)

    def slabs(ref, lo, n, rows=slice(None)):
        return jnp.concatenate([ref[lo + j, rows, :] for j in range(n)], axis=1)

    def wslabs(ref, lo, n, rows=slice(None)):
        return pltpu.bitcast(slabs(ref, lo, n, rows), bf16)

    def qk(Q, r0, ws, qs):
        out = []
        for w in ws:
            acc = None
            for j in range(NT):
                t = qs[j] * Q[NT + j, pl.ds(r0 + HALO - DIL * w, RC), :]
                acc = t if acc is None else acc + t
            out.append((acc, pltpu.roll(acc, 64, 1)))
        return out

    def ldq(Q, r0, z=None):
        qs = [Q[j, pl.ds(r0 + HALO, RC), :] for j in range(NT)]
        if z is not None:
            qs = [pltpu.bitcast(pltpu.bitcast(q, u32) | z, f32) for q in qs]
        return qs

    def stB(xs_):
        out = []
        for a, b in xs_:
            s_ = a + b
            out.append((s_, pltpu.roll(s_, 32, 1)))
        return out

    def stCD(Q, r0, xs_, masked, tile0, pg=None):
        ss = []
        for w, (a, b) in enumerate(xs_):
            acc = a + b
            if masked and w > 0:
                pos = tile0 + r0 + lax.broadcasted_iota(jnp.int32, (RC, 128), 0)
                acc = jnp.where(pos >= DIL * w, acc, -1e9 / (DH ** -0.5))
            ss.append(acc)
        m = functools.reduce(jnp.maximum, ss)
        ps = [jnp.exp2((s - m) * c2) for s in ss]
        den = functools.reduce(lambda a, b: a + b, ps)
        inv = 1.0 / den
        for j in range(NT):
            acc = None
            if pg is not None and pg(j) is not None:
                ps = [pltpu.bitcast(pltpu.bitcast(p_, u32) | pg(j), f32) for p_ in ps]
            for w in range(W):
                t = ps[w] * Q[2 * NT + j, pl.ds(r0 + HALO - DIL * w, RC), :]
                acc = t if acc is None else acc + t
            att_s[j, pl.ds(r0, RC), :] = acc * inv

    def attn_rows(Q, base, n, mode, tile0, grp, skew, gate=None, sub=None):
        r = lambda c: base + c * RC
        msk = lambda c: mode == 'all' or (mode == 'head' and c * RC < HALO)
        if grp:
            for c in range(n):
                qs = ldq(Q, r(c), gate(c) if gate else None)
                res = []
                for w0 in range(0, W, grp):
                    if sub and w0 and sub[0]:
                        qs = ldq(Q, r(c), gate(c + sub[0] * w0 / 4 / 100))
                    res += stB(qk(Q, r(c), range(w0, min(W, w0 + grp)), qs))
                pg = None
                if sub:
                    pg = lambda j: gate(c + (sub[1] + (sub[2] - sub[1]) * j / 4) / 100) if j % sub[3] == 0 and j >= sub[4] else None
                stCD(Q, r(c), res, msk(c), tile0, pg)
            return
        A, B = {}, {}
        for c in range(n + 2 * skew):
            if c < n:
                A[c] = qk(Q, r(c), range(W), ldq(Q, r(c), gate(c) if gate else None))
            if 0 <= c - skew < n:
                B[c - skew] = stB(A.pop(c - skew))
            if 0 <= c - 2 * skew < n:
                cc = c - 2 * skew
                stCD(Q, r(cc), B.pop(cc), msk(cc), tile0)

    def cp_x(t):
        rows = pl.ds(t * TM, TM)
        return pltpu.make_async_copy(x_hbm.at[rows, :], xin.at[rows, :], sem_x.at[0])
    def cp_o(t, lo=0, hi=D):
        rows = pl.ds(pl.multiple_of(t * TM, TM), TM)
        return pltpu.make_async_copy(obuf.at[rows, lo:hi], o_hbm.at[rows, lo:hi], sem_o.at[0])
    def cp_qkv(n):
        i = n // NT
        return pltpu.make_async_copy(wqkv_hbm.at[pl.ds(i % 2 * (D // 2), D // 2), pl.ds(i // 2 * D + n % NT * 128, 128)],
                                     stage.bitcast(bf16).at[n], sem_w.at[i % 3])
    def cp_wo(n):
        return pltpu.make_async_copy(wo_hbm.at[:, pl.ds(pl.multiple_of(n * 128, 128), 128)], stage_o.bitcast(bf16).at[n, 0:D, :], sem_m.at[n // 2])
    FGR = ((0, 1), (1, 2), (2, 4))
    def cp_w1(gr, j):
        return pltpu.make_async_copy(w1_hbm.at[:, pl.ds(j * 128, 128)], w1_ref.bitcast(bf16).at[j], sem_f.at[gr])
    def cp_w2(gr, j):
        rows = pl.ds(FGR[gr][0] * FC, (FGR[gr][1] - FGR[gr][0]) * FC)
        return pltpu.make_async_copy(w2_hbm.at[rows, pl.ds(j * 128, 128)], w2_ref.bitcast(bf16).at[j, rows, :], sem_f.at[gr])
    cp_b1 = pltpu.make_async_copy(b1_hbm, b1_v, sem_m.at[4])
    cp_b2 = pltpu.make_async_copy(b2_hbm, b2_v, sem_m.at[4])
    def wait_all(ref, sem):
        pltpu.make_async_copy(ref, ref, sem).wait()
    def wait_f(gr):
        lo, n = FGR[gr][0], FGR[gr][1] - FGR[gr][0]
        wait_all(w1_ref.at[pl.ds(lo * FC // 128, n * FC // 128)], sem_f.at[gr])
        wait_all(w2_ref.at[:, pl.ds(lo * FC // 2, n * FC // 2), :], sem_f.at[gr])

    def perm_cols(i, t):
        l = lax.broadcasted_iota(jnp.int32, (CR, 128), 1)
        u = (l >> 2) & 7
        X = [stage[i * NT + (v - t) % 8] for v in range(8)]
        for b in (4, 2, 1):
            X = [jnp.where((u & b) != 0, X[v + b], X[v]) for v in range(b)]
        w = jnp.take_along_axis(X[0], (l & 3) * 32 + ((u + t) & 7) * 4 + (l >> 5), axis=1)
        wqkv_ref[i // 2 * NT + t, pl.ds(pl.multiple_of(i % 2 * CR, CR), CR), :] = w
        return pltpu.bitcast(w, bf16)

    def perm_rows(n, gate):
        sub = lax.broadcasted_iota(jnp.int32, (8, 128), 0)
        def ld(base, o):
            v = stage_o[n, base + o:base + o + 8, :]
            if o > 8:
                v = jnp.where(sub < 16 - o, v, stage_o[n, base + o - 16:base + o - 8, :])
            return v
        for s_ in range(8):
            for hp in range(2):
                for m in range(2):
                    o = (2 * s_ + 8 * m) % 16
                    a_, b_ = ld(s_ * 64 + hp * 32, o), ld(s_ * 64 + hp * 32 + 16, o)
                    z = gate(s_ * 4 + hp * 2 + m)
                    if z is not None:
                        a_ = a_ | z
                    d0 = m * 256 + s_ * 2 + hp
                    wo_ref[n, pl.ds(d0, 8, stride=32), :] = (a_ & 0xffff) | (b_ << 16)
                    wo_ref[n, pl.ds(d0 + 16, 8, stride=32), :] = (a_ >> 16) | ((b_ >> 16) << 16)

    def zero_of(v):
        return (pltpu.bitcast(v, u32) >> 31) >> 1

    def ln_chunks(load, dst, lc, gate=None):
        for c in range(TM // lc):
            v = load(c * lc)
            if gate is not None:
                v = pltpu.bitcast(pltpu.bitcast(v, u32) | jnp.tile(gate(c), (lc // RC, NT)), f32)
            dst[c * (lc // 2):(c + 1) * (lc // 2), :] = pltpu.bitcast(_ln(v).astype(bf16), u32)

    def pick(tiles, t):
        j = int(t)
        i = int((t - j) * (TM // RC)) * RC
        return zero_of(tiles[j][i:i + RC, :])

    def cols(y):
        return [y[:, j * 128:(j + 1) * 128] for j in range(y.shape[1] // 128)]

    def starts(cp, lo, hi):
        for j in range(lo, hi):
            cp(j).start()
    def start_f1(gr):
        starts(lambda j: cp_w1(gr, j), FGR[gr][0] * FC // 128, FGR[gr][1] * FC // 128)
    def start_f2(gr):
        starts(lambda j: cp_w2(gr, j), 0, NT)

    cp_x(0).start(); starts(cp_qkv, 0, NT)
    qkv0_s[NT:, 0:HALO, :] = jnp.zeros((2 * NT, HALO, 128), f32)
    cp_x(0).wait()
    starts(cp_qkv, NT, 2 * NT)
    xn_s[...] = pltpu.bitcast(_ln(xin[0:TM, :].astype(f32)).astype(bf16), u32)
    NI = 6
    LI = 4
    LR = TM // (NI - LI)
    XI = 1
    WI = 3
    starts(cp_qkv, 2 * NT, 3 * NT)
    def wgrp(k):
        wait_all(stage.at[k * NT:(k + 1) * NT], sem_w.at[k % 3])
        if k == LI:
            cp_x(1).wait()
    def grp(k):
        starts(cp_qkv, (k + 3) * NT, min(k + 4, NI) * NT)
        if k == XI:
            cp_x(1).start()
        if WI <= k < WI + 2:
            starts(cp_wo, (k - WI) * 4, (k - WI + 1) * 4)
        if k == WI:
            cp_b1.start(); cp_b2.start()
        if k == NI - 1:
            start_f1(0); start_f2(0)
    def half(i, c2_):
        for k in range(NI):
            pl.when(i == k)(functools.partial(wgrp, k))
        p, kh = i // 2, i % 2
        a_ = pltpu.bitcast(xn_s[:, pl.ds(pl.multiple_of(kh * (D // 2), D // 2), D // 2)], bf16)
        ys = []
        for j in range(NT):
            ys.append(_dot(a_, perm_cols(i, j)))
            old = jnp.where(kh == 0, 0.0, qkv0_s[p * NT + j, HALO:HALO + TM, :])
            qkv0_s[p * NT + j, HALO:HALO + TM, :] = old + ys[j]
        def gt(f, span, off):
            t = f * span / 10 + off / 10
            return pick(ys, t) if t >= 0 else None
        src = pl.multiple_of(jnp.where(i < LI, 0, TM + (i - LI) * LR), LR)
        dst = pl.multiple_of(jnp.maximum(i - LI, 0) * (LR // 2), LR // 2)
        for c in range(LR // LC):
            v = xin[pl.ds(src + c * LC, LC), :].astype(f32)
            z = gt(c / (LR // LC), 40, 25)
            if z is not None:
                v = pltpu.bitcast(pltpu.bitcast(v, u32) | jnp.tile(z, (LC // RC, NT)), f32)
            xn2_s[pl.ds(dst + c * (LC // 2), LC // 2), :] = pltpu.bitcast(_ln(v).astype(bf16), u32)
        for k in range(NI):
            pl.when(i == k)(functools.partial(grp, k))
        return c2_
    lax.fori_loop(0, NI, half, 0)

    cp_b1.wait(); cp_b2.wait()
    b1_s[...] = b1_v[...].astype(f32).reshape(1, F)
    b2_s[...] = b2_v[...].astype(f32).reshape(1, D)
    qkv_s[NT:, 0:HALO, :] = qkv0_s[NT:, TM:TM + HALO, :]
    def grp2(k):
        if k == 0:
            start_f1(1); start_f2(1)
        if k == 1:
            start_f1(2)
        if k == 2:
            start_f2(2)
        if k == 3:
            starts(cp_x, 2, NTILE)
    def att(n, c1):
        wait_all(stage_o.at[pl.ds(2 * n, 2), 0:D // 2, :], sem_m.at[n])
        y = cols(_dot(pltpu.bitcast(xn2_s[...], bf16), wslabs(wqkv_ref, n * 6, 6)))
        for j in range(6):
            qkv_s[n * 6 + j, HALO:HALO + TM, :] = y[j]
        for k in range(4):
            pl.when(n == k)(functools.partial(grp2, k))
        PG = 55 / 10
        tq = lambda q: q // 2 * 2 * PG / 64 - 6 / 10
        for e in range(2):
            perm_rows(2 * n + e, lambda q: pick(y, tq(q + 32 * e)) if tq(q + 32 * e) >= 0 else None)
        attn_rows(qkv0_s, pl.multiple_of(n * (TM // 4), TM // 4), TM // 4 // RC, 'head', 0, GRP, SKEW,
                  lambda k: pick(y, (k * AG - AO) / 100) if k * AG >= AO else None, SUB)
        return c1
    lax.fori_loop(0, 4, att, 0)

    def step(g, carry):
        tp = (g + NTILE - 1) % NTILE
        rp = pl.multiple_of(tp * TM, TM)
        r = pl.multiple_of((g % NTILE) * TM, TM)
        edge = jnp.logical_or(g == 1, g == NJOB)

        def out_prev():
            @pl.when(g > NTILE + 1)
            def _():
                cp_o(g - NTILE - 2).start()

        def x_prev():
            return jnp.where(g <= NTILE, xin[pl.ds(rp, TM), :].astype(f32), xs[pl.ds(rp, TM), :])

        @pl.when(edge)
        def _():
            out_prev()
            for lo in (0, TM // 2):
                rows = pl.ds(rp + lo, TM // 2)
                xp = jnp.where(g <= NTILE, xin[rows, :].astype(f32), xs[rows, :])
                x2 = xp + _dot(slabs(att_s, 0, NT, slice(lo, lo + TM // 2)).astype(bf16), wslabs(wo_ref, 0, NT))
                xn2_s[lo // 2:lo // 2 + TM // 4, :] = pltpu.bitcast(_ln(x2).astype(bf16), u32)
                xs[rows, :] = x2 + b2_s[...]

        @pl.when(edge)
        def _():
            n = FC // 128
            nit = F // FC
            na = -(-(TM // RC) // nit)
            def ffn(c, c1):
                for gr in range(3):
                    pl.when(jnp.logical_and(g == 1, c == FGR[gr][0]))(functools.partial(wait_f, gr))
                @pl.when(jnp.logical_and(g == 1, c == nit - 1))
                def _():
                    wait_all(xin.at[2 * TM:S, :], sem_x.at[0])
                off = pl.multiple_of(c * FC, FC)
                h = _dot(pltpu.bitcast(xn2_s[...], bf16), wslabs(w1_ref, c * n, n)) + b1_s[:, pl.ds(off, FC)]
                hg = _gelu(h).astype(bf16)
                y = _dot(hg, wslabs(w2_ref, 0, NT, pl.ds(pl.multiple_of(c * (FC // 2), FC // 2), FC // 2)))
                x3 = xs[pl.ds(rp, TM), :] + y
                xs[pl.ds(rp, TM), :] = x3
                for lo, hi in zip(OC[:-1], OC[1:]):
                    obuf[pl.ds(rp, TM), lo:hi] = x3[:, lo:hi].astype(bf16)
                    if hi < D:
                        @pl.when(jnp.logical_and(g == NJOB, c == nit - 1))
                        def _():
                            cp_o(NTILE - 1, lo, hi).start()
                tl = cols(h) + cols(y)
                base = pl.multiple_of(jnp.minimum(c * na, TM // RC - na) * RC, RC)
                attn_rows(qkv_s, base, na, 'none', 0, GRP, SKEW, lambda k: pick(tl, F0 + k * FD / 100), SUB)
                return c1
            lax.fori_loop(0, nit, ffn, 0)

        @pl.when(jnp.logical_and(g > 1, g < NJOB))
        def _():
            yo = _dot(slabs(att_s, 0, NT).astype(bf16), wslabs(wo_ref, 0, NT))
            x2_s[...] = x_prev() + yo
            yos = cols(yo)
            nl = TM // LC
            ln_chunks(lambda o: jnp.where(g < NTILE, xin[pl.ds(r + o, LC), :].astype(f32), xs[pl.ds(r + o, LC), :]), xn_s, LC,
                      lambda c: pick(yos, c * G1 / 10 / nl))
            qkv_s[NT:, 0:HALO, :] = qkv_s[NT:, TM:TM + HALO, :]
            ys = cols(_dot(pltpu.bitcast(xn_s[...], bf16), wslabs(wqkv_ref, 0, 3 * NT)))
            for j in range(3 * NT):
                qkv_s[j, HALO:HALO + TM, :] = ys[j]
            ln_chunks(lambda o: x2_s[o:o + LC, :], xn2_s, LC, lambda c: pick(ys, c * G2 / nl))
            out_prev()
            h = _dot(pltpu.bitcast(xn2_s[...], bf16), wslabs(w1_ref, 0, NF)) + b1_s[...]
            hg = _gelu(h).astype(bf16)
            tl = cols(h)
            outs = []
            for j in range(NT):
                acc = None
                for k in range(F // 512):
                    t = _dot(hg[:, k * 512:(k + 1) * 512], wslabs(w2_ref, j, 1, slice(k * 256, (k + 1) * 256)))
                    acc = t if acc is None else acc + t
                    if (j * 7 + k) % 2 == 1:
                        tl.append(acc)
                outs.append(acc)
            x3 = x2_s[...] + jnp.concatenate(outs, axis=1) + b2_s[...]
            xs[pl.ds(rp, TM), :] = x3
            obuf[pl.ds(rp, TM), :] = x3.astype(bf16)
            na = TM // RC
            attn_rows(qkv_s, 0, na, 'head', r, GRP, SKEW, lambda c: pick(tl, A0 + c * (A1 - A0) / na), SUB)

        return carry

    lax.fori_loop(1, NJOB + 1, step, 0)
    cp_o(NTILE - 1, OC[-2], D).start()
    wait_all(obuf, sem_o.at[0])

@jax.jit
def pallas_interleave_layers__sliding_local_dilated__dense_activation_gelu__prompt_kernel(A_x, A_wqkv, A_wo, B_x, B_w1, B_b1, B_w2, B_b2):
    x = A_x.reshape(S, D)
    anyspec = pl.BlockSpec(memory_space=pl.ANY)
    V = pltpu.VMEM
    out = pl.pallas_call(
        kernel,
        in_specs=[anyspec] * 7,
        out_specs=anyspec,
        out_shape=jax.ShapeDtypeStruct((S, D), A_x.dtype),
        scratch_shapes=[V((S, D), bf16), V((S, D), bf16), V((S, D), f32), V((3 * NT, TM + HALO, 128), f32), V((3 * NT, TM + HALO, 128), f32), V((NT, TM, 128), f32),
            V((TM // 2, D), u32), V((TM // 2, D), u32), V((TM, D), f32),
            V((6 * NT, CR, 128), u32), V((NT, D // 2 + 8, 128), u32), V((F,), bf16), V((D,), bf16), V((1, F), f32), V((1, D), f32),
            V((3 * NT, D // 2, 128), u32), V((NT, D // 2, 128), u32), V((NF, D // 2, 128), u32), V((NT, F // 2, 128), u32),
            pltpu.SemaphoreType.DMA((1,)), pltpu.SemaphoreType.DMA((3,)), pltpu.SemaphoreType.DMA((5,)), pltpu.SemaphoreType.DMA((3,)), pltpu.SemaphoreType.DMA((1,))],
        compiler_params=pltpu.CompilerParams(vmem_limit_bytes=100 * 1024 * 1024),
    )(x, A_wqkv, A_wo, B_w1, B_b1, B_w2, B_b2)
    return out.reshape(1, S, D)
```

```python
import functools, math
import jax, jax.numpy as jnp
from jax import lax
import jax.experimental.pallas as pl
import jax.experimental.pallas.tpu as pltpu

S, D, F, H, DH, W, DIL = 2048, 1024, 3584, 32, 32, 8, 2
TM = 256
RC = 8
HALO = 16
NCH = 4
CR = D // NCH
SKEW = 1
GRP = 4
FU = 896
FC = 1792
LC = 16
OC = [128 * int(c) for c in "0578"]
AG = 73
AO = 60
F0 = 0
FD = 130
SUB = (25, 50, 75, 2, 1)
G1 = 60
G2 = 19
A0 = 3
A1 = 54
NT = D // 128
NF = F // 128
NTILE = S // TM
NJOB = 2 * NTILE
EPS = 1e-5
f32, bf16, u32 = jnp.float32, jnp.bfloat16, jnp.uint32

def _ln(x):
    m = jnp.mean(x, axis=-1, keepdims=True)
    xc = x - m
    v = jnp.mean(xc * xc, axis=-1, keepdims=True)
    return xc * lax.rsqrt(v + EPS)

def _gelu(x):
    c = math.sqrt(2.0 / math.pi)
    return 0.5 * x * (1.0 + jnp.tanh(c * (x + 0.044715 * (x * x * x))))

def _dot(a, b):
    return jnp.dot(a, b, preferred_element_type=f32)

def kernel(x_hbm, wqkv_hbm, wo_hbm, w1_hbm, b1_hbm, w2_hbm, b2_hbm, o_hbm,
           xin, obuf, xs, qkv_s, qkv0_s, att_s, xn_s, xn2_s, x2_s, stage, stage_o, b1_v, b2_v, b1_s, b2_s,
           wqkv_ref, wo_ref, w1_ref, w2_ref, sem_x, sem_w, sem_m, sem_f, sem_o):
    c2 = (DH ** -0.5) * math.log2(math.e)

    def slabs(ref, lo, n, rows=slice(None)):
        return jnp.concatenate([ref[lo + j, rows, :] for j in range(n)], axis=1)

    def wslabs(ref, lo, n, rows=slice(None)):
        return pltpu.bitcast(slabs(ref, lo, n, rows), bf16)

    def qk(Q, r0, ws, qs):
        out = []
        for w in ws:
            acc = None
            for j in range(NT):
                t = qs[j] * Q[NT + j, pl.ds(r0 + HALO - DIL * w, RC), :]
                acc = t if acc is None else acc + t
            out.append((acc, pltpu.roll(acc, 64, 1)))
        return out

    def ldq(Q, r0, z=None):
        qs = [Q[j, pl.ds(r0 + HALO, RC), :] for j in range(NT)]
        if z is not None:
            qs = [pltpu.bitcast(pltpu.bitcast(q, u32) | z, f32) for q in qs]
        return qs

    def stB(xs_):
        out = []
        for a, b in xs_:
            s_ = a + b
            out.append((s_, pltpu.roll(s_, 32, 1)))
        return out

    def stCD(Q, r0, xs_, masked, tile0, pg=None):
        ss = []
        for w, (a, b) in enumerate(xs_):
            acc = a + b
            if masked and w > 0:
                pos = tile0 + r0 + lax.broadcasted_iota(jnp.int32, (RC, 128), 0)
                acc = jnp.where(pos >= DIL * w, acc, -1e9 / (DH ** -0.5))
            ss.append(acc)
        m = functools.reduce(jnp.maximum, ss)
        ps = [jnp.exp2((s - m) * c2) for s in ss]
        den = functools.reduce(lambda a, b: a + b, ps)
        inv = 1.0 / den
        for j in range(NT):
            acc = None
            if pg is not None and pg(j) is not None:
                ps = [pltpu.bitcast(pltpu.bitcast(p_, u32) | pg(j), f32) for p_ in ps]
            for w in range(W):
                t = ps[w] * Q[2 * NT + j, pl.ds(r0 + HALO - DIL * w, RC), :]
                acc = t if acc is None else acc + t
            att_s[j, pl.ds(r0, RC), :] = acc * inv

    def attn_rows(Q, base, n, mode, tile0, grp, skew, gate=None, sub=None):
        r = lambda c: base + c * RC
        msk = lambda c: mode == 'all' or (mode == 'head' and c * RC < HALO)
        if grp:
            for c in range(n):
                qs = ldq(Q, r(c), gate(c) if gate else None)
                res = []
                for w0 in range(0, W, grp):
                    if sub and w0 and sub[0]:
                        qs = ldq(Q, r(c), gate(c + sub[0] * w0 / 4 / 100))
                    res += stB(qk(Q, r(c), range(w0, min(W, w0 + grp)), qs))
                pg = None
                if sub:
                    pg = lambda j: gate(c + (sub[1] + (sub[2] - sub[1]) * j / 4) / 100) if j % sub[3] == 0 and j >= sub[4] else None
                stCD(Q, r(c), res, msk(c), tile0, pg)
            return
        A, B = {}, {}
        for c in range(n + 2 * skew):
            if c < n:
                A[c] = qk(Q, r(c), range(W), ldq(Q, r(c), gate(c) if gate else None))
            if 0 <= c - skew < n:
                B[c - skew] = stB(A.pop(c - skew))
            if 0 <= c - 2 * skew < n:
                cc = c - 2 * skew
                stCD(Q, r(cc), B.pop(cc), msk(cc), tile0)

    def cp_x(t):
        rows = pl.ds(t * TM, TM)
        return pltpu.make_async_copy(x_hbm.at[rows, :], xin.at[rows, :], sem_x.at[0])
    def cp_o(t, lo=0, hi=D):
        rows = pl.ds(pl.multiple_of(t * TM, TM), TM)
        return pltpu.make_async_copy(obuf.at[rows, lo:hi], o_hbm.at[rows, lo:hi], sem_o.at[0])
    def cp_qkv(n):
        i = n // NT
        return pltpu.make_async_copy(wqkv_hbm.at[pl.ds(i % 2 * (D // 2), D // 2), pl.ds(i // 2 * D + n % NT * 128, 128)],
                                     stage.bitcast(bf16).at[n], sem_w.at[i % 3])
    def cp_wo(n):
        return pltpu.make_async_copy(wo_hbm.at[:, pl.ds(pl.multiple_of(n * 128, 128), 128)], stage_o.bitcast(bf16).at[n, 0:D, :], sem_m.at[n // 4])
    FGR = ((0, 1), (1, 2), (2, 4))
    def cp_w1(gr, j):
        return pltpu.make_async_copy(w1_hbm.at[:, pl.ds(j * 128, 128)], w1_ref.bitcast(bf16).at[j], sem_f.at[gr])
    def cp_w2(gr, j):
        rows = pl.ds(FGR[gr][0] * FU, (FGR[gr][1] - FGR[gr][0]) * FU)
        return pltpu.make_async_copy(w2_hbm.at[rows, pl.ds(j * 128, 128)], w2_ref.bitcast(bf16).at[j, rows, :], sem_f.at[3 + gr])
    cp_b1 = pltpu.make_async_copy(b1_hbm, b1_v, sem_m.at[2])
    cp_b2 = pltpu.make_async_copy(b2_hbm, b2_v, sem_m.at[2])
    def wait_all(ref, sem):
        pltpu.make_async_copy(ref, ref, sem).wait()
    def wait_f(gr):
        lo, n = FGR[gr][0], FGR[gr][1] - FGR[gr][0]
        wait_all(w1_ref.at[pl.ds(lo * FU // 128, n * FU // 128)], sem_f.at[gr])
        wait_all(w2_ref.at[:, pl.ds(lo * FU // 2, n * FU // 2), :], sem_f.at[3 + gr])

    def perm_cols(i, t):
        l = lax.broadcasted_iota(jnp.int32, (CR, 128), 1)
        u = (l >> 2) & 7
        X = [stage[i * NT + (v - t) % 8] for v in range(8)]
        for b in (4, 2, 1):
            X = [jnp.where((u & b) != 0, X[v + b], X[v]) for v in range(b)]
        w = jnp.take_along_axis(X[0], (l & 3) * 32 + ((u + t) & 7) * 4 + (l >> 5), axis=1)
        wqkv_ref[i // 2 * NT + t, pl.ds(pl.multiple_of(i % 2 * CR, CR), CR), :] = w
        return pltpu.bitcast(w, bf16)

    def perm_rows(n, gate):
        sub = lax.broadcasted_iota(jnp.int32, (8, 128), 0)
        def ld(base, o):
            v = stage_o[n, base + o:base + o + 8, :]
            if o > 8:
                v = jnp.where(sub < 16 - o, v, stage_o[n, base + o - 16:base + o - 8, :])
            return v
        for s_ in range(8):
            for hp in range(2):
                for m in range(2):
                    o = (2 * s_ + 8 * m) % 16
                    a_, b_ = ld(s_ * 64 + hp * 32, o), ld(s_ * 64 + hp * 32 + 16, o)
                    z = gate(s_ * 4 + hp * 2 + m)
                    if z is not None:
                        a_ = a_ | z
                    d0 = m * 256 + s_ * 2 + hp
                    wo_ref[n, pl.ds(d0, 8, stride=32), :] = (a_ & 0xffff) | (b_ << 16)
                    wo_ref[n, pl.ds(d0 + 16, 8, stride=32), :] = (a_ >> 16) | ((b_ >> 16) << 16)

    def zero_of(v):
        return (pltpu.bitcast(v, u32) >> 31) >> 1

    def ln_chunks(load, dst, lc, gate=None):
        for c in range(TM // lc):
            v = load(c * lc)
            if gate is not None:
                v = pltpu.bitcast(pltpu.bitcast(v, u32) | jnp.tile(gate(c), (lc // RC, NT)), f32)
            dst[c * (lc // 2):(c + 1) * (lc // 2), :] = pltpu.bitcast(_ln(v).astype(bf16), u32)

    def pick(tiles, t):
        j = int(t)
        i = int((t - j) * (TM // RC)) * RC
        return zero_of(tiles[j][i:i + RC, :])

    def cols(y):
        return [y[:, j * 128:(j + 1) * 128] for j in range(y.shape[1] // 128)]

    def starts(cp, lo, hi):
        for j in range(lo, hi):
            cp(j).start()
    def start_f1(gr):
        starts(lambda j: cp_w1(gr, j), FGR[gr][0] * FU // 128, FGR[gr][1] * FU // 128)
    def start_f2(gr):
        starts(lambda j: cp_w2(gr, j), 0, NT)

    cp_x(0).start(); starts(cp_qkv, 0, NT)
    qkv0_s[NT:, 0:HALO, :] = jnp.zeros((2 * NT, HALO, 128), f32)
    cp_x(0).wait()
    starts(cp_qkv, NT, 2 * NT)
    xn_s[...] = pltpu.bitcast(_ln(xin[0:TM, :].astype(f32)).astype(bf16), u32)
    NI = 6
    LI = 4
    LR = TM // (NI - LI)
    XI = 1
    WI = 3
    starts(cp_qkv, 2 * NT, 3 * NT)
    def wgrp(k):
        wait_all(stage.at[k * NT:(k + 1) * NT], sem_w.at[k % 3])
        if k == LI:
            cp_x(1).wait()
    def grp(k):
        starts(cp_qkv, (k + 3) * NT, min(k + 4, NI) * NT)
        if k == XI:
            cp_x(1).start()
        if WI <= k < WI + 2:
            starts(cp_wo, (k - WI) * 4, (k - WI + 1) * 4)
        if k == WI:
            cp_b1.start(); cp_b2.start()
        if k == NI - 1:
            start_f1(0); start_f2(0)
    def half(i, c2_):
        for k in range(NI):
            pl.when(i == k)(functools.partial(wgrp, k))
        p, kh = i // 2, i % 2
        a_ = pltpu.bitcast(xn_s[:, pl.ds(pl.multiple_of(kh * (D // 2), D // 2), D // 2)], bf16)
        ys = []
        for j in range(NT):
            ys.append(_dot(a_, perm_cols(i, j)))
            old = jnp.where(kh == 0, 0.0, qkv0_s[p * NT + j, HALO:HALO + TM, :])
            qkv0_s[p * NT + j, HALO:HALO + TM, :] = old + ys[j]
        def gt(f, span, off):
            t = f * span / 10 + off / 10
            return pick(ys, t) if t >= 0 else None
        src = pl.multiple_of(jnp.where(i < LI, 0, TM + (i - LI) * LR), LR)
        dst = pl.multiple_of(jnp.maximum(i - LI, 0) * (LR // 2), LR // 2)
        for c in range(LR // LC):
            v = xin[pl.ds(src + c * LC, LC), :].astype(f32)
            z = gt(c / (LR // LC), 40, 25)
            if z is not None:
                v = pltpu.bitcast(pltpu.bitcast(v, u32) | jnp.tile(z, (LC // RC, NT)), f32)
            xn2_s[pl.ds(dst + c * (LC // 2), LC // 2), :] = pltpu.bitcast(_ln(v).astype(bf16), u32)
        for k in range(NI):
            pl.when(i == k)(functools.partial(grp, k))
        return c2_
    lax.fori_loop(0, NI, half, 0)

    cp_b1.wait(); cp_b2.wait()
    b1_s[...] = b1_v[...].astype(f32).reshape(1, F)
    b2_s[...] = b2_v[...].astype(f32).reshape(1, D)
    qkv_s[NT:, 0:HALO, :] = qkv0_s[NT:, TM:TM + HALO, :]
    start_f1(1); start_f2(1)
    def att(n, c1):
        wait_all(stage_o.at[pl.ds(4 * n, 4), 0:D // 2, :], sem_m.at[n])
        y = cols(_dot(pltpu.bitcast(xn2_s[...], bf16), wslabs(wqkv_ref, n * 12, 12)))
        for j in range(12):
            qkv_s[n * 12 + j, HALO:HALO + TM, :] = y[j]
        pl.when(n == 0)(functools.partial(start_f1, 2))
        pl.when(n < 1)(functools.partial(start_f2, 2))
        tq = lambda q: q // 2 * 2 * 115 / 10 / 128 - 6 / 10
        for e in range(4):
            perm_rows(4 * n + e, lambda q: pick(y, tq(q + 32 * e)) if tq(q + 32 * e) >= 0 else None)
        attn_rows(qkv0_s, pl.multiple_of(n * (TM // 2), TM // 2), TM // 2 // RC, 'head', 0, GRP, SKEW,
                  lambda k: pick(y, (k * AG - AO) / 100) if k * AG >= AO else None, SUB)
        return c1
    lax.fori_loop(0, 2, att, 0)
    starts(cp_x, 2, NTILE)

    def step(g, carry):
        tp = (g + NTILE - 1) % NTILE
        rp = pl.multiple_of(tp * TM, TM)
        r = pl.multiple_of((g % NTILE) * TM, TM)
        edge = jnp.logical_or(g == 1, g == NJOB)

        def out_prev():
            @pl.when(g > NTILE + 1)
            def _():
                cp_o(g - NTILE - 2).start()

        def x_prev():
            return jnp.where(g <= NTILE, xin[pl.ds(rp, TM), :].astype(f32), xs[pl.ds(rp, TM), :])

        @pl.when(edge)
        def _():
            out_prev()
            for lo in (0, TM // 2):
                rows = pl.ds(rp + lo, TM // 2)
                xp = jnp.where(g <= NTILE, xin[rows, :].astype(f32), xs[rows, :])
                x2 = xp + _dot(slabs(att_s, 0, NT, slice(lo, lo + TM // 2)).astype(bf16), wslabs(wo_ref, 0, NT))
                xn2_s[lo // 2:lo // 2 + TM // 4, :] = pltpu.bitcast(_ln(x2).astype(bf16), u32)
                xs[rows, :] = x2 + b2_s[...]

        @pl.when(edge)
        def _():
            n = FC // 128
            nit = F // FC
            na = -(-(TM // RC) // nit)
            def ffn(c, c1):
                for gr in range(3):
                    pl.when(jnp.logical_and(g == 1, c == FGR[gr][0] * FU // FC))(functools.partial(wait_f, gr))
                off = pl.multiple_of(c * FC, FC)
                h = _dot(pltpu.bitcast(xn2_s[...], bf16), wslabs(w1_ref, c * n, n)) + b1_s[:, pl.ds(off, FC)]
                hg = _gelu(h).astype(bf16)
                y = _dot(hg, wslabs(w2_ref, 0, NT, pl.ds(pl.multiple_of(c * (FC // 2), FC // 2), FC // 2)))
                x3 = xs[pl.ds(rp, TM), :] + y
                xs[pl.ds(rp, TM), :] = x3
                for lo, hi in zip(OC[:-1], OC[1:]):
                    obuf[pl.ds(rp, TM), lo:hi] = x3[:, lo:hi].astype(bf16)
                    if hi < D:
                        @pl.when(jnp.logical_and(g == NJOB, c == nit - 1))
                        def _():
                            cp_o(NTILE - 1, lo, hi).start()
                tl = cols(h) + cols(y)
                base = pl.multiple_of(jnp.minimum(c * na, TM // RC - na) * RC, RC)
                attn_rows(qkv_s, base, na, 'none', 0, GRP, SKEW, lambda k: pick(tl, F0 + k * FD / 100), SUB)
                return c1
            lax.fori_loop(0, nit, ffn, 0)
            @pl.when(g == 1)
            def _():
                wait_all(xin.at[2 * TM:S, :], sem_x.at[0])

        @pl.when(jnp.logical_and(g > 1, g < NJOB))
        def _():
            yo = _dot(slabs(att_s, 0, NT).astype(bf16), wslabs(wo_ref, 0, NT))
            x2_s[...] = x_prev() + yo
            yos = cols(yo)
            nl = TM // LC
            ln_chunks(lambda o: jnp.where(g < NTILE, xin[pl.ds(r + o, LC), :].astype(f32), xs[pl.ds(r + o, LC), :]), xn_s, LC,
                      lambda c: pick(yos, c * G1 / 10 / nl))
            qkv_s[NT:, 0:HALO, :] = qkv_s[NT:, TM:TM + HALO, :]
            ys = cols(_dot(pltpu.bitcast(xn_s[...], bf16), wslabs(wqkv_ref, 0, 3 * NT)))
            for j in range(3 * NT):
                qkv_s[j, HALO:HALO + TM, :] = ys[j]
            ln_chunks(lambda o: x2_s[o:o + LC, :], xn2_s, LC, lambda c: pick(ys, c * G2 / nl))
            out_prev()
            h = _dot(pltpu.bitcast(xn2_s[...], bf16), wslabs(w1_ref, 0, NF)) + b1_s[...]
            hg = _gelu(h).astype(bf16)
            tl = cols(h)
            outs = []
            for j in range(NT):
                acc = None
                for k in range(F // 512):
                    t = _dot(hg[:, k * 512:(k + 1) * 512], wslabs(w2_ref, j, 1, slice(k * 256, (k + 1) * 256)))
                    acc = t if acc is None else acc + t
                    if (j * 7 + k) % 2 == 1:
                        tl.append(acc)
                outs.append(acc)
            x3 = x2_s[...] + jnp.concatenate(outs, axis=1) + b2_s[...]
            xs[pl.ds(rp, TM), :] = x3
            obuf[pl.ds(rp, TM), :] = x3.astype(bf16)
            na = TM // RC
            attn_rows(qkv_s, 0, na, 'head', r, GRP, SKEW, lambda c: pick(tl, A0 + c * (A1 - A0) / na), SUB)

        return carry

    lax.fori_loop(1, NJOB + 1, step, 0)
    cp_o(NTILE - 1, OC[-2], D).start()
    wait_all(obuf, sem_o.at[0])

@jax.jit
def pallas_interleave_layers__sliding_local_dilated__dense_activation_gelu__prompt_kernel(A_x, A_wqkv, A_wo, B_x, B_w1, B_b1, B_w2, B_b2):
    x = A_x.reshape(S, D)
    anyspec = pl.BlockSpec(memory_space=pl.ANY)
    V = pltpu.VMEM
    out = pl.pallas_call(
        kernel,
        in_specs=[anyspec] * 7,
        out_specs=anyspec,
        out_shape=jax.ShapeDtypeStruct((S, D), A_x.dtype),
        scratch_shapes=[V((S, D), bf16), V((S, D), bf16), V((S, D), f32), V((3 * NT, TM + HALO, 128), f32), V((3 * NT, TM + HALO, 128), f32), V((NT, TM, 128), f32),
            V((TM // 2, D), u32), V((TM // 2, D), u32), V((TM, D), f32),
            V((6 * NT, CR, 128), u32), V((NT, D // 2 + 8, 128), u32), V((F,), bf16), V((D,), bf16), V((1, F), f32), V((1, D), f32),
            V((3 * NT, D // 2, 128), u32), V((NT, D // 2, 128), u32), V((NF, D // 2, 128), u32), V((NT, F // 2, 128), u32),
            pltpu.SemaphoreType.DMA((1,)), pltpu.SemaphoreType.DMA((3,)), pltpu.SemaphoreType.DMA((3,)), pltpu.SemaphoreType.DMA((6,)), pltpu.SemaphoreType.DMA((1,))],
        compiler_params=pltpu.CompilerParams(vmem_limit_bytes=100 * 1024 * 1024),
    )(x, A_wqkv, A_wo, B_w1, B_b1, B_w2, B_b2)
    return out.reshape(1, S, D)
```
